```python
import os as _os
_os.environ.setdefault('JAX_PLATFORMS', 'cpu')
import jax
import jax.numpy as jnp

def _softmax(x, axis=-1):
    return jax.nn.softmax(x, axis=axis)

def _gelu(x):
    return jax.nn.gelu(x, approximate=True)

def _silu(x):
    return jax.nn.silu(x)

def _sigmoid(x):
    return jax.nn.sigmoid(x)

def _layernorm(x, axis=-1, eps=1e-05):
    m = jnp.mean(x, axis=axis, keepdims=True)
    v = jnp.var(x, axis=axis, keepdims=True)
    return (x - m) / jnp.sqrt(v + eps)

def _scatter_add(tgt, idx, src, axis=0):
    return tgt.at[idx].add(src)

def _segment_sum(src, seg, n):
    return jax.ops.segment_sum(src, seg, n)

class _Rng:

    def __init__(self, key):
        self._k = key

    def _next(self):
        self._k, sub = jax.random.split(self._k)
        return sub

    def normal(self, shape):
        return jax.random.normal(self._next(), shape, dtype=jnp.bfloat16)

    def randint(self, lo, hi, shape):
        return jax.random.randint(self._next(), shape, lo, hi, dtype=jnp.int32)

    def uniform(self, shape, lo=0.0, hi=1.0):
        return jax.random.uniform(self._next(), shape, jnp.bfloat16, lo, hi)

    def permutation(self, n):
        return jax.random.permutation(self._next(), n)
kernel_name = 'gated_mix__grouped_kv_mqa__memory_aug_recurrent_mem_tr__prompt'

def setup_inputs():
    _rng = _Rng(jax.random.key(int.from_bytes(__import__("os").urandom(4), "little")))
    _w = lambda a: (lambda t: t.astype(jnp.bfloat16) if jnp.issubdtype(t.dtype, jnp.floating) else t)(jnp.asarray(a))

    def _A_setup():
        B, S, D, H = (1, 2048, 1024, 32)
        Dh = D // H
        return {'x': _w((lambda *s: _rng.normal(s) * 0.05)(B, S, D)), 'wq': _w((lambda *s: _rng.normal(s) * 1.6)(D, H * Dh)), 'wk': _w((lambda *s: _rng.normal(s) * 1.6)(D, Dh)), 'wv': _w((lambda *s: _rng.normal(s) * 0.05)(D, Dh)), 'wo': _w((lambda *s: _rng.normal(s) * 0.05)(H * Dh, D))}
    _A_in = _A_setup()

    def _B_setup():
        B, S, Dm = (1, 2048, 1024)
        H, Dh = (32, 128)
        M, seg = (8, 32)
        seg = min(seg, S)
        S = S // seg * seg
        return {'x': _w((lambda *s: _rng.normal(s) * 0.05)(B, S, Dm)), 'mem0': _w((lambda *s: _rng.normal(s) * 0.8)(B, M, Dm)), 'Wq': _w((lambda *s: _rng.normal(s) * 3.2)(Dm, H, Dh) * Dm ** (-0.5)), 'Wk': _w((lambda *s: _rng.normal(s) * 3.2)(Dm, H, Dh) * Dm ** (-0.5)), 'Wv': _w((lambda *s: _rng.normal(s) * 0.8)(Dm, H, Dh) * Dm ** (-0.5)), 'Wo': _w((lambda *s: _rng.normal(s) * 0.8)(H, Dh, Dm) * (H * Dh) ** (-0.5)), 'seg_len': seg}
    _B_in = _B_setup()
    return {'A_x': _A_in['x'], 'A_wq': _A_in['wq'], 'A_wk': _A_in['wk'], 'A_wv': _A_in['wv'], 'A_wo': _A_in['wo'], 'B_x': _B_in['x'], 'B_mem0': _B_in['mem0'], 'B_Wq': _B_in['Wq'], 'B_Wk': _B_in['Wk'], 'B_Wv': _B_in['Wv'], 'B_Wo': _B_in['Wo'], 'B_seg_len': _B_in['seg_len'], 'gate_w': _w((lambda *s: _rng.normal(s) * 0.05)(1024) * 16.0)}

def reference(A_x, A_wq, A_wk, A_wv, A_wo, B_x, B_mem0, B_Wq, B_Wk, B_Wv, B_Wo, B_seg_len, gate_w):

    def _A_ref(x, wq, wk, wv, wo):
        B, S, D = x.shape
        H = 32
        Dh = D // H
        q = (lambda x, *d: x.transpose(*d))((x @ wq).reshape(B, S, H, Dh), 0, 2, 1, 3)
        k = x @ wk
        v = x @ wv
        scores = jnp.einsum('bhqd,bkd->bhqk', q, k) * Dh ** (-0.5)
        p = _softmax(scores, axis=-1)
        o = jnp.einsum('bhqk,bkd->bhqd', p, v)
        return (lambda x, *d: x.transpose(*d))(o, 0, 2, 1, 3).reshape(B, S, H * Dh) @ wo

    def _B_ref(x, mem0, Wq, Wk, Wv, Wo, seg_len):
        B, S, Dm = x.shape
        H, Dh = (Wq.shape[1], Wq.shape[2])
        M = mem0.shape[1]
        scale = Dh ** (-0.5)
        n_seg = S // seg_len
        L = M + seg_len
        idx = jnp.arange(L)
        mask = (idx[:, None] < M) | (idx[:, None] >= idx[None, :])
        mem = mem0
        outs = []
        for s in range(n_seg):
            xs = x[:, s * seg_len:(s + 1) * seg_len, :].copy()
            h = jnp.concatenate([mem, xs], axis=1)
            q = jnp.einsum('btd,dhe->bhte', h, Wq)
            k = jnp.einsum('btd,dhe->bhte', h, Wk)
            v = jnp.einsum('btd,dhe->bhte', h, Wv)
            scores = jnp.einsum('bhqe,bhke->bhqk', q, k) * scale
            scores = jnp.where(mask[None, None], scores, -1000000000.0)
            p = _softmax(scores, axis=-1)
            o = jnp.einsum('bhqk,bhke->bhqe', p, v)
            o = jnp.einsum('bhte,hed->btd', o, Wo)
            mem = o[:, :M, :].copy()
            outs.append(o[:, M:, :])
        return jnp.concatenate(outs, axis=1)
    x = A_x
    g = _sigmoid((x * gate_w).sum(-1, keepdims=True))
    a = _A_ref(x, A_wq, A_wk, A_wv, A_wo)
    b = _B_ref(x, B_mem0, B_Wq, B_Wk, B_Wv, B_Wo, B_seg_len)
    return g * a + (1 - g) * b
```

```python
import functools
import math

import jax
import jax.numpy as jnp
import jax.experimental.pallas as pl
import jax.experimental.pallas.tpu as pltpu

F32 = jnp.float32
BF16 = jnp.bfloat16
U32 = jnp.uint32

S = 2048
D = 1024
HA = 32
DHA = 32
HB = 32
DHB = 128
M = 8
SEG = 32
NSEG = S // SEG
L = M + SEG
NUNIT = (S // 128) * (D // 128)
CH = 256
NCH = S // CH
NT = (((1,), (1,)), ((), ()))


def _dot(a, b):
    return jnp.dot(a, b, preferred_element_type=F32)


def _kernel(x_hbm, wqa_hbm, wka_ref, wva_ref, woa_hbm, mem0_ref, wq_hbm, wk_hbm,
            wv_hbm, wo_hbm, gw_ref, out_hbm,
            x_v, wqa_v, woa_v, wqkv_v, wo_v, qt_v, ka_v, vt_v, g_v, qkv0_v,
            land_v, st_v, m_v, ocat_v, o0_v, b_v, oa_v, out_v,
            sem_x, sem_wa, sem_w, sem_wo, sem_out):
    XC = 4
    xs = NSEG // XC

    def x_copy(i):
        return pltpu.make_async_copy(x_hbm.at[pl.ds(i * xs, xs)],
                                     x_v.at[pl.ds(i * xs, xs)], sem_x.at[i])

    wqa_copy = pltpu.make_async_copy(wqa_hbm, wqa_v, sem_wa.at[0])
    woa_copy = pltpu.make_async_copy(woa_hbm, woa_v, sem_wa.at[1])
    w_hbms = (wq_hbm, wk_hbm, wv_hbm)

    def w_copy(i):
        return pltpu.make_async_copy(w_hbms[i], land_v.at[i], sem_w.at[i])

    def wo_copy(c):
        return pltpu.make_async_copy(wo_hbm.at[:, pl.ds(c * 128, 128)],
                                     wo_v.at[c], sem_wo.at[c])

    wqa_copy.start()
    for i in range(XC):
        x_copy(i).start()
    for i in range(3):
        w_copy(i).start()
    for c in range(8):
        wo_copy(c).start()
    woa_copy.start()

    qscale = (DHA ** -0.5) * math.log2(math.e)
    wkv = jnp.concatenate(
        [wka_ref[...], wva_ref[...], jnp.zeros((D, 128 - 2 * DHA), BF16)], axis=1)
    gw = gw_ref[...].astype(F32)

    def aproj(rb):
        xb = x_v[pl.ds(rb * 4, 4)].reshape(128, D)
        q = _dot(xb, wqa_v[...]) * qscale
        qT = q.T.astype(BF16)
        for b in range(8):
            for j in range(4):
                r = b * 128 + j * 32
                qt_v[rb * 8 + b, :, j * 128:(j + 1) * 128] = qT[r:r + 32, :]
        kv = _dot(xb, wkv)
        r0 = pl.multiple_of(rb * 128, 128)
        ka_v[pl.ds(r0, 128), :] = kv[:, :DHA].astype(BF16)
        vt_v[:, pl.ds(r0, 128)] = kv.T[DHA:2 * DHA, :].astype(BF16)
        z = jnp.sum(xb.astype(F32) * gw, axis=1, keepdims=True)
        g_v[pl.ds(r0, 128), :] = jax.nn.sigmoid(z)

    def relayout(i, g):
        v = land_v[i, pl.ds(pl.multiple_of(g * 2048, 2048), 2048), :]
        t = jnp.transpose(v.reshape(64, HB, DHB), (1, 0, 2))
        wqkv_v[i, :, pl.ds(pl.multiple_of(g * 32, 32), 32), :] = pltpu.bitcast(t, U32)

    def wblk(i, h):
        return pltpu.bitcast(wqkv_v[i, h], BF16)

    wqa_copy.wait()
    for i in range(XC):
        x_copy(i).wait()

        def abody(t, c, i=i):
            aproj(i * 4 + t)
            return c
        jax.lax.fori_loop(0, 4, abody, 0)

    w_copy(0).wait()

    def rbody0(g, c):
        relayout(0, g)
        return c
    jax.lax.fori_loop(0, 16, rbody0, 0)

    for i in range(3):
        if i < 2:
            w_copy(i + 1).wait()

        def bbody(g, c, i=i):
            x0 = x_v[:, 0:M, :].reshape(NSEG * M, D)
            for hh in range(2):
                h = g * 2 + hh
                qkv0_v[i, h] = _dot(x0, wblk(i, h)).astype(BF16)
            if i < 2:
                relayout(i + 1, g)
            return c
        jax.lax.fori_loop(0, 16, bbody, 0)

    for c in range(8):
        wo_copy(c).wait()
    x_v[0, 0:M, :] = mem0_ref[...]

    def qk_chunk(u, slot, c, mx):
        st = _dot(ka_v[c * CH:(c + 1) * CH, :], qt_v[u])
        st_v[slot, c * CH:(c + 1) * CH, :] = st
        cm = jnp.max(st.reshape(CH // 8, 8, 512), axis=0)
        return cm if mx is None else jnp.maximum(mx, cm)

    def pv_chunk(slot, c, m, l, acc):
        p = jnp.exp2(st_v[slot, c * CH:(c + 1) * CH, :] - m)
        cl = jnp.sum(p.reshape(CH // 8, 8, 512), axis=0)
        o = _dot(vt_v[:, c * CH:(c + 1) * CH], p.astype(BF16))
        return (cl if l is None else l + cl), (o if acc is None else acc + o)

    def a_finish(u, l, acc):
        o = acc / jnp.sum(l, axis=0, keepdims=True)
        o4 = jnp.concatenate([o[:, j * 128:(j + 1) * 128] for j in range(4)], axis=0)
        qb = u // 8
        b = u % 8
        oa_v[pl.ds(pl.multiple_of(qb * 128, 128), 128),
             pl.ds(pl.multiple_of(b * 128, 128), 128)] = o4.T.astype(BF16)

    mx = None
    for c in range(NCH):
        mx = qk_chunk(0, 0, c, mx)
    m_v[...] = jnp.max(mx, axis=0, keepdims=True)

    ri = jax.lax.broadcasted_iota(jnp.int32, (L, L), 0)
    ci = jax.lax.broadcasted_iota(jnp.int32, (L, L), 1)

    def pos(i):
        return jnp.where(i < M, i, jnp.where(i < SEG, i + M, i - SEG + M))
    mask = (ri < M) | (pos(ri) >= pos(ci))
    bscale = DHB ** -0.5

    def step(s, carry):
        h = x_v[s]
        r0 = pl.multiple_of(s * M, M)

        class A:
            m = m_v[...]
            mx = None
            l = None
            acc = None
            n = 0

        def a_work():
            t, c = divmod(A.n, NCH)
            u = s * 2 + t
            A.mx = qk_chunk(jnp.minimum(u + 1, NUNIT - 1), 1 - t, c, A.mx)
            A.l, A.acc = pv_chunk(t, c, A.m, A.l, A.acc)
            if c == NCH - 1:
                a_finish(u, A.l, A.acc)
                A.m = jnp.max(A.mx, axis=0, keepdims=True)
                A.mx = A.l = A.acc = None
            A.n += 1

        def proj(hd):
            return [_dot(h, wblk(i, hd)).astype(BF16) for i in range(3)]

        def attn(hd, qkv):
            q, k, v = [jnp.concatenate([qkv[i], qkv0_v[i, hd, pl.ds(r0, M), :]], axis=0)
                       for i in range(3)]
            sc = jax.lax.dot_general(q, k, NT, preferred_element_type=F32) * bscale
            sc = jnp.where(mask, sc, -1000000000.0)
            p = jnp.exp(sc - jnp.max(sc, axis=1, keepdims=True))
            l = jnp.sum(p, axis=1, keepdims=True)
            o = (_dot(p.astype(BF16), v) / l).astype(BF16)
            ocat_v[:, hd * 128:(hd + 1) * 128] = o[:SEG]
            o0_v[pl.ds(r0, M), hd * 128:(hd + 1) * 128] = o[SEG:]

        G = 4
        prev = None
        for g in range(HB // G):
            cur = [proj(g * G + j) for j in range(G)]
            if prev is not None:
                for j in range(G):
                    attn((g - 1) * G + j, prev[j])
            a_work()
            prev = cur
        a_work()
        for j in range(G):
            attn(HB - G + j, prev[j])
        for _ in range(3):
            a_work()
        oc = ocat_v[...]
        ys = [_dot(oc, wo_v[c]) for c in range(8)]
        y = jnp.concatenate(ys, axis=1)
        b_v[s, M:, :] = y[M:]
        x_v[jnp.minimum(s + 1, NSEG - 1), 0:M, :] = y[:M].astype(BF16)
        for _ in range(4):
            a_work()
        m_v[...] = A.m
        return carry

    jax.lax.fori_loop(0, NSEG, step, 0)

    woa_copy.wait()
    o0 = o0_v[...]
    for c in range(8):
        b_v[:, 0:M, c * 128:(c + 1) * 128] = _dot(o0, wo_v[c]).reshape(NSEG, M, 128)

    EB = 256
    NEB = S // EB

    def out_copy(i):
        return pltpu.make_async_copy(out_v.at[pl.ds(i * EB, EB)],
                                     out_hbm.at[pl.ds(i * EB, EB)], sem_out.at[i])

    for i in range(NEB):
        a = _dot(oa_v[i * EB:(i + 1) * EB, :], woa_v[...])
        b = b_v[i * (EB // SEG):(i + 1) * (EB // SEG)].reshape(EB, D)
        g = g_v[i * EB:(i + 1) * EB, :]
        out_v[i * EB:(i + 1) * EB, :] = (g * a + (1.0 - g) * b).astype(BF16)
        out_copy(i).start()
    for i in range(NEB):
        out_copy(i).wait()


@functools.partial(jax.jit, static_argnames=("B_seg_len",))
def pallas_gated_mix__grouped_kv_mqa__memory_aug_recurrent_mem_tr__prompt_kernel(
    A_x, A_wq, A_wk, A_wv, A_wo, B_x, B_mem0, B_Wq, B_Wk, B_Wv, B_Wo, B_seg_len,
    gate_w,
):
    del B_x
    assert B_seg_len == SEG and A_x.shape == (1, S, D)
    hbm = pl.BlockSpec(memory_space=pl.ANY)
    vmem = pl.BlockSpec(memory_space=pltpu.VMEM)
    out = pl.pallas_call(
        _kernel,
        out_shape=jax.ShapeDtypeStruct((S, D), BF16),
        in_specs=[hbm, hbm, vmem, vmem, hbm, vmem, hbm, hbm, hbm, hbm, vmem],
        out_specs=hbm,
        scratch_shapes=[
            pltpu.VMEM((NSEG, SEG, D), BF16),
            pltpu.VMEM((D, D), BF16),
            pltpu.VMEM((D, D), BF16),
            pltpu.VMEM((3, HB, D // 2, DHB), U32),
            pltpu.VMEM((8, HB * DHB, 128), BF16),
            pltpu.VMEM((NUNIT, DHA, 512), BF16),
            pltpu.VMEM((S, DHA), BF16),
            pltpu.VMEM((DHA, S), BF16),
            pltpu.VMEM((S, 1), F32),
            pltpu.VMEM((3, HB, NSEG * M, DHB), BF16),
            pltpu.VMEM((3, D * HB, DHB), BF16),
            pltpu.VMEM((2, S, 512), F32),
            pltpu.VMEM((1, 512), F32),
            pltpu.VMEM((SEG, HB * DHB), BF16),
            pltpu.VMEM((NSEG * M, HB * DHB), BF16),
            pltpu.VMEM((NSEG, SEG, D), F32),
            pltpu.VMEM((S, D), BF16),
            pltpu.VMEM((S, D), BF16),
            pltpu.SemaphoreType.DMA((4,)),
            pltpu.SemaphoreType.DMA((2,)),
            pltpu.SemaphoreType.DMA((3,)),
            pltpu.SemaphoreType.DMA((8,)),
            pltpu.SemaphoreType.DMA((8,)),
        ],
        compiler_params=pltpu.CompilerParams(vmem_limit_bytes=124 * 1024 * 1024),
    )(
        A_x.reshape(NSEG, SEG, D), A_wq, A_wk, A_wv, A_wo, B_mem0.reshape(M, D),
        B_Wq.reshape(D * HB, DHB), B_Wk.reshape(D * HB, DHB),
        B_Wv.reshape(D * HB, DHB), B_Wo.reshape(HB * DHB, D),
        gate_w.reshape(1, D),
    )
    return out.reshape(1, S, D)
```

```python
import functools
import math

import jax
import jax.numpy as jnp
import jax.experimental.pallas as pl
import jax.experimental.pallas.tpu as pltpu

F32 = jnp.float32
BF16 = jnp.bfloat16
U32 = jnp.uint32

S = 2048
D = 1024
DHA = 32
HB = 32
DHB = 128
M = 8
SEG = 32
NSEG = S // SEG
L = M + SEG
NUNIT = (S // 128) * (D // 128)
CH = 256
NCH = S // CH
NIT = 2 * NCH
NT = (((1,), (1,)), ((), ()))
NEG = -1000000000.0
NSTEPS = NSEG
A_AFTER_PART = [1,3,4,6,7,9,10,12,13,15,16,17]
A_AFTER_WO = [2,5]
GQ_AFTER_PART = [16,17,22,25]
GP_AFTER_PART = [17,22,25,27]
QL = 10
WQC = 2
DM = 1
MDEP = 1


def _dot(a, b):
    return jnp.dot(a, b, preferred_element_type=F32)


def _dot_nt(a, b):
    return jax.lax.dot_general(a, b, NT, preferred_element_type=F32)


def _recip(x):
    return pl.reciprocal(x, approx=False, full_range=False)


def _kernel(x_hbm, wqa_hbm, wka_hbm, wva_hbm, woa_hbm, mem0_hbm, wq_hbm, wk_hbm,
            wv_hbm, wo_hbm, gw_hbm, out_hbm,
            x_v, wqa_v, woa_v, wkvz_v, gw_v, mem0_v, wq_v, wk_v, wv_v, wo_v,
            qt_v, ka_v, vt_v, g_v, q0_v, k0_v, v0_v, km_v, vm_v, lq_v, lk_v, lv_v,
            sg0_v, sg1_v, st_v, mx_v, fin_v, ocat_v, o0_v, o7_v, b_v, oa_v, out_v,
            sem_x, sem_s, sem_wa, sem_w, sem_wo, sem_out):
    XC = 4
    xs = NSEG // XC
    w_hbms = (wq_hbm, wk_hbm, wv_hbm)
    w_vs = (wq_v, wk_v, wv_v)
    land_vs = (lq_v, lk_v, lv_v)
    qkv0_vs = (q0_v, k0_v, v0_v)
    stg_vs = (sg0_v, sg1_v)

    def x_copy(i):
        return pltpu.make_async_copy(x_hbm.at[pl.ds(i * xs, xs)],
                                     x_v.at[pl.ds(i * xs, xs)], sem_x.at[i])

    small = [
        pltpu.make_async_copy(wka_hbm, wkvz_v.at[pl.ds(0, DHA)], sem_s.at[0]),
        pltpu.make_async_copy(wva_hbm, wkvz_v.at[pl.ds(DHA, DHA)], sem_s.at[1]),
        pltpu.make_async_copy(gw_hbm, gw_v, sem_s.at[2]),
        pltpu.make_async_copy(mem0_hbm, mem0_v, sem_s.at[3]),
    ]

    def wqa_copy(c):
        cs = pl.ds(c * (D // WQC), D // WQC)
        return pltpu.make_async_copy(wqa_hbm.at[:, cs], wqa_v.at[:, cs], sem_wa.at[c])

    woa_copy = pltpu.make_async_copy(woa_hbm, woa_v, sem_wa.at[4])

    def w_copy(i):
        return pltpu.make_async_copy(w_hbms[i], land_vs[i], sem_w.at[i])

    def wo_copy(c):
        return pltpu.make_async_copy(wo_hbm.at[:, pl.ds(c * 128, 128)],
                                     lq_v.at[pl.ds(c * HB * DHB, HB * DHB)],
                                     sem_wo.at[c])

    x_copy(0).start()
    for cp in small:
        cp.start()
    for c in range(WQC):
        wqa_copy(c).start()

    km_v[:, 0:64, :] = jnp.zeros((HB, 64, DHB), BF16)
    vm_v[:, 0:64, :] = jnp.zeros((HB, 64, DHB), BF16)

    qscale = (DHA ** -0.5) * math.log2(math.e)

    def xblk(rb):
        return x_v[pl.ds(rb * 4, 4)].reshape(128, D)

    def aproj_kvz(rb):
        kvz = _dot_nt(wkvz_v[...], xblk(rb))
        r0 = pl.multiple_of(rb * 128, 128)
        vt_v[:, pl.ds(r0, 128)] = kvz[DHA:2 * DHA, :].astype(BF16)
        t = jnp.concatenate([kvz, jnp.zeros((48, 128), F32)], axis=0).T
        ka_v[pl.ds(r0, 128), :] = t[:, :DHA].astype(BF16)
        g_v[pl.ds(r0, 128), :] = jnp.broadcast_to(
            jax.nn.sigmoid(t[:, 2 * DHA:2 * DHA + 1]), (128, 128))

    def aproj_q(rb, b):
        q = _dot(xblk(rb), wqa_v[:, b * 128:(b + 1) * 128]) * qscale
        qT = q.T.astype(BF16)
        for j in range(4):
            qt_v[rb * 8 + b, :, j * 128:(j + 1) * 128] = qT[j * 32:(j + 1) * 32, :]

    def aproj(rb, extra=()):
        extra = list(extra)
        aproj_kvz(rb)
        for b in range(8):
            aproj_q(rb, b)
            if extra:
                extra.pop(0)()

    def relayout(i, g):
        for blk in range(2):
            stg = stg_vs[blk]
            base = pl.multiple_of(g * 1024 + blk * 512, 512)
            v = pltpu.bitcast(land_vs[i][pl.ds(base, 512), :], U32)
            for k in range(8):
                a = v[32 * k:32 * k + 16]
                b = v[32 * k + 16:32 * k + 32]
                stg[pl.ds(3 * k, 16, stride=25), :] = (a & U32(0xffff)) | (b << 16)
                stg[pl.ds(400 + 3 * k, 16, stride=25), :] = (a >> 16) | (b & U32(0xffff0000))
            r = pl.multiple_of(g * 16 + blk * 8, 8)
            for p in range(16):
                w_vs[i][2 * p, pl.ds(r, 8), :] = stg[pl.ds(25 * p, 8, stride=3), :]
                w_vs[i][2 * p + 1, pl.ds(r, 8), :] = stg[pl.ds(400 + 25 * p, 8, stride=3), :]

    def wo_pack(g):
        v = lq_v[pl.ds(pl.multiple_of(g * 1024, 1024), 1024), :]
        wo_v[pl.ds(pl.multiple_of(g * 512, 512), 512), :] = pltpu.bitcast(v, U32)

    def wblk(i, h):
        return pltpu.bitcast(w_vs[i][h], BF16)

    def woblk(c):
        return pltpu.bitcast(wo_v[c * 2048:(c + 1) * 2048, :], BF16)

    for cp in small:
        cp.wait()
    gw = gw_v[...]
    gw_row = jnp.concatenate([gw[r:r + 1, :] for r in range(8)], axis=1)
    wkvz_v[2 * DHA:, :] = jnp.broadcast_to(gw_row, (16, D))
    x_copy(0).wait()
    for i in range(1, XC):
        x_copy(i).start()
    w_copy(0).start()
    if DM == 1:
        w_copy(1).start()
    for rb in range(4):
        aproj_kvz(rb)
    for c in range(WQC):
        wqa_copy(c).wait()
        for rb in range(4):
            for b in range(c * (8 // WQC), (c + 1) * (8 // WQC)):
                aproj_q(rb, b)

    def abody0(t, c):
        aproj(t * 2)
        aproj(t * 2 + 1)
        return c
    for i in range(1, 3):
        x_copy(i).wait()
        if DM == 2 and i == 2:
            w_copy(1).start()
        jax.lax.fori_loop(2 * i, 2 * i + 2, abody0, 0)
    x_copy(3).wait()
    w_copy(0).wait()
    if DM == 0:
        w_copy(1).start()
    w_copy(2).start()

    def abody1(t, c):
        for k in range(2):
            g0 = t * 16 + k * 8
            aproj(12 + t * 2 + k,
                  [functools.partial(relayout, 0, g0 + r) for r in range(8)])
        return c
    jax.lax.fori_loop(0, 2, abody1, 0)

    for i in range(3):
        if i < 2:
            w_copy(i + 1).wait()
        if i == 0:
            for c in range(8):
                wo_copy(c).start()
            woa_copy.start()
        if i == 2:
            for c in range(8):
                wo_copy(c).wait()

        def bbody(g, c, i=i):
            for hh in range(8):
                h = g * 8 + hh
                x0 = x_v[:, 0:M, :].reshape(NSEG * M, D)
                qkv0_vs[i][h] = _dot(x0, wblk(i, h)).astype(BF16)
                if i < 2:
                    relayout(i + 1, h)
                else:
                    wo_pack(h)
            return c
        jax.lax.fori_loop(0, 4, bbody, 0)

    x_v[0, 0:M, :] = mem0_v[...]

    def qk_chunk(u, slot, c, mx):
        st = _dot(ka_v[c * CH:(c + 1) * CH, :], qt_v[u])
        st_v[slot, c * CH:(c + 1) * CH, :] = st
        cm = jnp.max(st.reshape(CH // 8, 8, 512), axis=0)
        return cm if mx is None else jnp.maximum(mx, cm)

    def pv_exp(slot, c, m8):
        st = st_v[slot, c * CH:(c + 1) * CH, :].reshape(CH // 8, 8, 512)
        p = jnp.exp2(st - m8[None])
        pk = p.reshape(CH, 512).astype(BF16)
        while p.shape[0] > 1:
            p = p.reshape(p.shape[0] // 2, 2, 8, 512)
            p = p[:, 0] + p[:, 1]
        return p[0], pk

    def colmax(mx):
        return jnp.broadcast_to(jnp.max(mx, axis=0, keepdims=True), (8, 512))

    def a_finish(u, l, acc):
        o = acc * _recip(jnp.sum(l, axis=0, keepdims=True))
        o4 = jnp.concatenate([o[:, j * 128:(j + 1) * 128] for j in range(4)], axis=0)
        qb = u // 8
        b = u % 8
        oa_v[pl.ds(pl.multiple_of(qb * 128, 128), 128),
             pl.ds(pl.multiple_of(b * 128, 128), 128)] = o4.T.astype(BF16)

    mxs = [None, None]
    for n in range(QL):
        t, c = divmod(n, NCH)
        mxs[t] = qk_chunk(t, t, c, mxs[t])
    mx_v[0] = mxs[0]
    mx_v[1] = mxs[1]
    fin_v[...] = jnp.ones((40, 512), F32)

    bscale = DHB ** -0.5
    ri = jax.lax.broadcasted_iota(jnp.int32, (SEG, L), 0)
    ci = jax.lax.broadcasted_iota(jnp.int32, (SEG, L), 1)
    mask = (ri < M) | (ci >= SEG) | (ri >= ci)
    gr = jax.lax.broadcasted_iota(jnp.int32, (64, 128), 0)
    gc = jax.lax.broadcasted_iota(jnp.int32, (64, 128), 1)
    gsame = (gr // M) == ((gc % 64) // M)
    gmask = gsame & ((gc < 64) | (gr >= gc - 64))

    def softmax_nonorm(sc):
        p = jnp.exp(sc - jnp.max(sc, axis=1, keepdims=True))
        return p.astype(BF16), _recip(jnp.sum(p, axis=1, keepdims=True))

    def grp_qk(grp, hd):
        rs = pl.ds(pl.multiple_of(grp * 64, 64), 64)
        k = jnp.concatenate([km_v[hd, rs, :], k0_v[hd, rs, :]], axis=0)
        sc = _dot_nt(q0_v[hd, rs, :], k) * bscale
        sc = jnp.where(gmask, sc, jnp.where(gsame, NEG, -jnp.inf))
        return softmax_nonorm(sc)

    def grp_pv(grp, hd, pr, last=False):
        rs = pl.ds(pl.multiple_of(grp * 64, 64), 64)
        v = jnp.concatenate([vm_v[hd, rs, :], v0_v[hd, rs, :]], axis=0)
        o = (_dot(pr[0], v) * pr[1]).astype(BF16)
        cs = pl.ds(pl.multiple_of(hd * 128, 128), 128)
        if last:
            o7_v[:, cs] = o
        else:
            o0_v[rs, cs] = o

    def step(s, carry):
        h = x_v[s]
        r0 = pl.multiple_of(s * M, M)
        grp = jnp.maximum(s // 8 - 1, 0)
        gh0 = (s % 8) * 4

        mx = {0: mx_v[0], 1: mx_v[1]}
        m8 = {0: colmax(mx[0])}
        ls = {}
        acc = {}
        pks = {}
        mhist = {}

        def a_exp(n):
            t, c = divmod(n, NCH)
            m = m8[t]
            if n - MDEP in mhist:
                dep = mhist[n - MDEP]
                m = jnp.where(dep > jnp.inf, dep, m)
            cl, pks[n] = pv_exp(t % 2, c, m)
            ls[t] = cl if t not in ls else ls[t] + cl

        def a_item(j):
            t, c = divmod(j + QL, NCH)
            u = jnp.minimum(s * 2 + t, NUNIT - 1)
            mx[t] = qk_chunk(u, t % 2, c, mx.get(t))
            if c == NCH - 1:
                m8[t] = colmax(mx[t])
            t, c = divmod(j, NCH)
            o = _dot(vt_v[:, c * CH:(c + 1) * CH], pks.pop(j))
            acc[t] = o if t not in acc else acc[t] + o
            mhist[j] = o[0:8]
            if j == NCH - 1:
                a_finish(s * 2, ls[0], acc[0])
            if j + 1 < NIT:
                a_exp(j + 1)

        def proj(hd):
            q, k, v = [_dot(h, wblk(i, hd)).astype(BF16) for i in range(3)]
            km_v[hd, pl.ds(r0, M), :] = k[:M]
            vm_v[hd, pl.ds(r0, M), :] = v[:M]
            return q, k, v

        def attn_qk(hd, qkv):
            q, k, v = qkv
            k = jnp.concatenate([k, k0_v[hd, pl.ds(r0, M), :]], axis=0)
            v = jnp.concatenate([v, v0_v[hd, pl.ds(r0, M), :]], axis=0)
            sc = jnp.where(mask, _dot_nt(q, k) * bscale, NEG)
            return softmax_nonorm(sc) + (v,)

        def attn_pv(hd, prv):
            p, r, v = prv
            o = (_dot(p, v) * r).astype(BF16)
            ocat_v[:, hd * 128:(hd + 1) * 128] = pltpu.bitcast(o, U32)

        def g_work(k):
            for j in range(4):
                if GP_AFTER_PART[j] == k:
                    grp_pv(grp, gh0 + j, gps.pop(j))
            for j in range(4):
                if GQ_AFTER_PART[j] == k:
                    gps[j] = grp_qk(grp, gh0 + j)

        a_finish(jnp.maximum(s * 2 - 1, 0), fin_v[32:40, :], fin_v[0:32, :])
        a_exp(0)
        projs = {}
        pvs = {}
        gps = {}
        g_work(-1)
        na = 0
        NP = HB // 2
        for k in range(NP + 2):
            if k < NP:
                for j in range(2):
                    projs[2 * k + j] = proj(2 * k + j)
            if k >= 2:
                for j in range(2):
                    hd = 2 * (k - 2) + j
                    attn_pv(hd, pvs.pop(hd))
            if 1 <= k <= NP:
                for j in range(2):
                    hd = 2 * (k - 1) + j
                    pvs[hd] = attn_qk(hd, projs.pop(hd))
            g_work(k)
            if k in A_AFTER_PART:
                a_item(na)
                na += 1
        oc = pltpu.bitcast(ocat_v[...], BF16)
        ys = []
        for c in range(8):
            ys.append(_dot(oc, woblk(c)))
            g_work(20 + c)
            if c in A_AFTER_WO:
                a_item(na)
                na += 1
        y = jnp.concatenate(ys, axis=1)
        b_v[s, M:, :] = y[M:]
        x_v[jnp.minimum(s + 1, NSEG - 1), 0:M, :] = y[:M].astype(BF16)
        while na < NIT:
            a_item(na)
            na += 1
        mx_v[0] = mx[2]
        mx_v[1] = mx[3]
        fin_v[0:32, :] = acc[1]
        fin_v[32:40, :] = ls[1]
        return carry

    jax.lax.fori_loop(0, NSTEPS, step, 0)

    a_finish(NUNIT - 1, fin_v[32:40, :], fin_v[0:32, :])
    woa_copy.wait()
    EB = 256
    NEB = S // EB

    def out_copy(i):
        return pltpu.make_async_copy(out_v.at[pl.ds(i * EB, EB)],
                                     out_hbm.at[pl.ds(i * EB, EB)], sem_out.at[i])

    def eblock(i, nlast):
        r0 = pl.multiple_of(i * EB, EB)
        s0 = pl.multiple_of(i * 8, 8)
        o0 = o0_v[pl.ds(pl.multiple_of(i * 64, 64), 64), :]
        oa = oa_v[pl.ds(r0, EB), :]
        gps = {}
        for c in range(8):
            cs = slice(c * 128, (c + 1) * 128)
            b0 = _dot(o0, woblk(c)).reshape(8, M, 128)
            b = jnp.concatenate([b0, b_v[pl.ds(s0, 8), M:, cs]], axis=1).reshape(EB, 128)
            if nlast and 1 <= c <= 4:
                for j in (2 * c - 2, 2 * c - 1):
                    grp_pv(7, i * 8 + j, gps.pop(j), True)
            a = _dot(oa, woa_v[:, cs])
            g = g_v[pl.ds(r0, EB), :]
            out_v[pl.ds(r0, EB), cs] = (g * a + (1.0 - g) * b).astype(BF16)
            if nlast and c < 4:
                for j in (2 * c, 2 * c + 1):
                    gps[j] = grp_qk(7, i * 8 + j)
        out_copy(i).start()

    def ebody0(i, carry):
        eblock(i, 8)
        return carry

    def ebody1(i, carry):
        eblock(i, 0)
        return carry
    jax.lax.fori_loop(0, 4, ebody0, 0)
    o0_v[pl.ds(7 * 64, 64), :] = o7_v[...]
    jax.lax.fori_loop(4, NEB, ebody1, 0)
    for i in range(NEB):
        out_copy(i).wait()


@functools.partial(jax.jit, static_argnames=("B_seg_len",))
def pallas_gated_mix__grouped_kv_mqa__memory_aug_recurrent_mem_tr__prompt_kernel(
    A_x, A_wq, A_wk, A_wv, A_wo, B_x, B_mem0, B_Wq, B_Wk, B_Wv, B_Wo, B_seg_len,
    gate_w,
):
    del B_x
    assert B_seg_len == SEG and A_x.shape == (1, S, D)
    hbm = pl.BlockSpec(memory_space=pl.ANY)
    wsc = pltpu.VMEM((HB, D // 2, DHB), U32)
    p0sc = pltpu.VMEM((HB, NSEG * M, DHB), BF16)
    lsc = pltpu.VMEM((D * HB, DHB), BF16)
    out = pl.pallas_call(
        _kernel,
        out_shape=jax.ShapeDtypeStruct((S, D), BF16),
        in_specs=[hbm] * 11,
        out_specs=hbm,
        scratch_shapes=[
            pltpu.VMEM((NSEG, SEG, D), BF16),
            pltpu.VMEM((D, D), BF16),
            pltpu.VMEM((D, D), BF16),
            pltpu.VMEM((80, D), BF16),
            pltpu.VMEM((8, 128), BF16),
            pltpu.VMEM((M, D), BF16),
            wsc, wsc, wsc,
            pltpu.VMEM((8 * HB * DHB // 2, 128), U32),
            pltpu.VMEM((NUNIT, DHA, 512), BF16),
            pltpu.VMEM((S, DHA), BF16),
            pltpu.VMEM((DHA, S), BF16),
            pltpu.VMEM((S, 128), F32),
            p0sc, p0sc, p0sc,
            p0sc, p0sc,
            lsc, lsc, lsc,
            pltpu.VMEM((800, 128), U32),
            pltpu.VMEM((800, 128), U32),
            pltpu.VMEM((2, S, 512), F32),
            pltpu.VMEM((2, 8, 512), F32),
            pltpu.VMEM((40, 512), F32),
            pltpu.VMEM((SEG // 2, HB * DHB), U32),
            pltpu.VMEM((NSEG * M, HB * DHB), BF16),
            pltpu.VMEM((64, HB * DHB), BF16),
            pltpu.VMEM((NSEG, SEG, D), F32),
            pltpu.VMEM((S, D), BF16),
            pltpu.VMEM((S, D), BF16),
            pltpu.SemaphoreType.DMA((4,)),
            pltpu.SemaphoreType.DMA((4,)),
            pltpu.SemaphoreType.DMA((5,)),
            pltpu.SemaphoreType.DMA((3,)),
            pltpu.SemaphoreType.DMA((8,)),
            pltpu.SemaphoreType.DMA((8,)),
        ],
        compiler_params=pltpu.CompilerParams(vmem_limit_bytes=127 * 1024 * 1024),
    )(
        A_x.reshape(NSEG, SEG, D), A_wq, A_wk.T, A_wv.T, A_wo, B_mem0.reshape(M, D),
        B_Wq.reshape(D * HB, DHB), B_Wk.reshape(D * HB, DHB),
        B_Wv.reshape(D * HB, DHB), B_Wo.reshape(HB * DHB, D),
        gate_w.reshape(8, 128),
    )
    return out.reshape(1, S, D)
```

```python
import functools
import math

import jax
import jax.numpy as jnp
import jax.experimental.pallas as pl
import jax.experimental.pallas.tpu as pltpu

F32 = jnp.float32
BF16 = jnp.bfloat16
U32 = jnp.uint32

S = 2048
D = 1024
DHA = 32
HB = 32
DHB = 128
M = 8
SEG = 32
NSEG = S // SEG
L = M + SEG
NUNIT = (S // 128) * (D // 128)
CH = 256
NCH = S // CH
NIT = 2 * NCH
NT = (((1,), (1,)), ((), ()))
NEG = -1000000000.0
NSTEPS = NSEG
A_AFTER_PART = [1,3,4,6,7,9,10,12,13,15,16,17]
A_AFTER_WO = [1,4,6]
GQ_AFTER_PART = [17,21,23,25]
GP_AFTER_PART = [21,23,25,27]
QL = 10
WQC = 2
DM = 1
NPC = 8
MARGIN = 1
LEAD = 12
WOS = 4
UNROLL = 2
MDEP = 1


def _dot(a, b):
    return jnp.dot(a, b, preferred_element_type=F32)


def _dot_nt(a, b):
    return jax.lax.dot_general(a, b, NT, preferred_element_type=F32)


def _recip(x):
    return pl.reciprocal(x, approx=False, full_range=False)


def _kernel(x_hbm, wqa_hbm, wka_hbm, wva_hbm, woa_hbm, mem0_hbm, wq_hbm, wk_hbm,
            wv_hbm, wo_hbm, gw_hbm, out_hbm,
            x_v, x0_v, wqa_v, woa_v, wkvz_v, gw_v, mem0_v, wq_v, wk_v, wv_v, wo_v,
            qt_v, ka_v, vt_v, g_v, q0_v, k0_v, v0_v, lq_v, lk_v, lv_v,
            sg0_v, sg1_v, st_v, mx_v, fin_v, ocat_v, o0_v, o7_v, b_v, oa_v,
            sem_x, sem_s, sem_wa, sem_w, sem_wo, sem_out):
    XC = 4
    xs = NSEG // XC
    w_hbms = (wq_hbm, wk_hbm, wv_hbm)
    w_vs = (wq_v, wk_v, wv_v)
    land_vs = (lq_v, lk_v, lv_v)
    qkv0_vs = (q0_v, k0_v, v0_v)
    stg_vs = (sg0_v, sg1_v)

    def x_copy(i):
        return pltpu.make_async_copy(x_hbm.at[pl.ds(i * xs, xs)],
                                     x_v.at[pl.ds(i * xs, xs)], sem_x.at[i])

    small = [
        pltpu.make_async_copy(wka_hbm, wkvz_v.at[pl.ds(0, DHA)], sem_s.at[0]),
        pltpu.make_async_copy(wva_hbm, wkvz_v.at[pl.ds(DHA, DHA)], sem_s.at[1]),
        pltpu.make_async_copy(gw_hbm, gw_v, sem_s.at[2]),
        pltpu.make_async_copy(mem0_hbm, mem0_v, sem_s.at[3]),
    ]

    def wqa_copy(c):
        cs = pl.ds(c * (D // WQC), D // WQC)
        return pltpu.make_async_copy(wqa_hbm.at[:, cs], wqa_v.at[:, cs], sem_wa.at[c])

    woa_copy = pltpu.make_async_copy(woa_hbm, woa_v, sem_wa.at[4])

    def w_copy(i):
        return pltpu.make_async_copy(w_hbms[i], land_vs[i], sem_w.at[i])

    def wq_copy(j):
        rs = pl.ds(j * (D * HB // 2), D * HB // 2)
        return pltpu.make_async_copy(wq_hbm.at[rs], lq_v.at[rs], sem_w.at[3 * j])

    def wo_copy(c):
        return pltpu.make_async_copy(wo_hbm.at[:, pl.ds(c * 128, 128)],
                                     lq_v.at[pl.ds(c * HB * DHB, HB * DHB)],
                                     sem_wo.at[c])

    x_copy(0).start()
    for cp in small:
        cp.start()
    for c in range(WQC):
        wqa_copy(c).start()

    def kvm_rows(kv, hd, r, n):
        return pl.ds(pl.multiple_of((kv * HB + hd) * (NSEG * M) + r, M), n)

    qscale = (DHA ** -0.5) * math.log2(math.e)

    def xblk(rb):
        return x_v[pl.ds(rb * 4, 4)].reshape(128, D)

    def aproj_kvz(rb):
        kvz = _dot_nt(wkvz_v[...], xblk(rb))
        r0 = pl.multiple_of(rb * 128, 128)
        vt_v[:, pl.ds(r0, 128)] = kvz[DHA:2 * DHA, :].astype(BF16)
        t = jnp.concatenate([kvz, jnp.zeros((48, 128), F32)], axis=0).T
        ka_v[pl.ds(r0, 128), :] = t[:, :DHA].astype(BF16)
        x0 = x_v[pl.ds(rb * 4, 4), 0:M, :].reshape(4 * M, D)
        x0_v[pl.ds(pl.multiple_of(rb * 16, 16), 16), :] = pltpu.bitcast(x0, U32)
        g_v[pl.ds(r0, 128), :] = jnp.broadcast_to(
            jax.nn.sigmoid(t[:, 2 * DHA:2 * DHA + 1]), (128, 128))

    def aproj_q(rb, b):
        q = _dot(xblk(rb), wqa_v[:, b * 128:(b + 1) * 128]) * qscale
        qT = q.T.astype(BF16)
        for j in range(4):
            qt_v[rb * 8 + b, :, j * 128:(j + 1) * 128] = qT[j * 32:(j + 1) * 32, :]
        return q[0:16]

    def aproj(rb, extra=()):
        extra = list(extra)
        aproj_kvz(rb)
        for b in range(8):
            dep = aproj_q(rb, b)
            if extra:
                extra.pop(0)(dep=dep)

    def relayout(i, g, blks=(0, 1), dep=None):
        for blk in blks:
            stg = stg_vs[blk]
            base = pl.multiple_of(g * 1024 + blk * 512, 512)
            v = pltpu.bitcast(land_vs[i][pl.ds(base, 512), :], U32)
            for k in range(8):
                a = v[32 * k:32 * k + 16]
                b = v[32 * k + 16:32 * k + 32]
                if dep is not None:
                    a = jnp.where(dep > jnp.inf, U32(0), a)
                stg[pl.ds(3 * k, 16, stride=25), :] = (a & U32(0xffff)) | (b << 16)
                stg[pl.ds(400 + 3 * k, 16, stride=25), :] = (a >> 16) | (b & U32(0xffff0000))
            r = pl.multiple_of(g * 16 + blk * 8, 8)
            for p in range(16):
                w_vs[i][2 * p, pl.ds(r, 8), :] = stg[pl.ds(25 * p, 8, stride=3), :]
                w_vs[i][2 * p + 1, pl.ds(r, 8), :] = stg[pl.ds(400 + 25 * p, 8, stride=3), :]

    def wo_pack(g):
        v = lq_v[pl.ds(pl.multiple_of(g * 1024, 1024), 1024), :]
        wo_v[pl.ds(pl.multiple_of(g * 512, 512), 512), :] = pltpu.bitcast(v, U32)

    def wblk(i, h):
        return pltpu.bitcast(w_vs[i][h], BF16)

    def woblk(c):
        return pltpu.bitcast(wo_v[c * 2048:(c + 1) * 2048, :], BF16)

    for cp in small:
        cp.wait()
    gw = gw_v[...]
    gw_row = jnp.concatenate([gw[r:r + 1, :] for r in range(8)], axis=1)
    wkvz_v[2 * DHA:, :] = jnp.broadcast_to(gw_row, (16, D))
    x_copy(0).wait()
    for i in range(1, XC):
        x_copy(i).start()
    wq_copy(0).start()
    wq_copy(1).start()
    w_copy(1).start()
    for rb in range(4):
        aproj_kvz(rb)
    for c in range(WQC):
        wqa_copy(c).wait()
        for rb in range(4):
            for b in range(c * (8 // WQC), (c + 1) * (8 // WQC)):
                aproj_q(rb, b)

    def abody0(t, c):
        aproj(t * 2)
        aproj(t * 2 + 1)
        return c
    x_copy(1).wait()
    jax.lax.fori_loop(2, 4, abody0, 0)
    x_copy(2).wait()
    wq_copy(0).wait()

    def abody1(t, c):
        @pl.when(t == 2)
        def _():
            x_copy(3).wait()
            wq_copy(1).wait()
            w_copy(2).start()
        for k in range(2):
            g0 = t * 8 + k * 4
            aproj(8 + t * 2 + k,
                  [functools.partial(relayout, 0, g0 + r // 2, (r % 2,))
                   for r in range(8)])
        return c
    jax.lax.fori_loop(0, 4, abody1, 0)

    for i in range(3):
        if i < 2:
            w_copy(i + 1).wait()
        if i == 0:
            for c in range(8):
                wo_copy(c).start()
            woa_copy.start()
        if i == 2:
            for c in range(8):
                wo_copy(c).wait()

        def bbody(g, c, i=i):
            for hh in range(8):
                h = g * 8 + hh
                x0 = pltpu.bitcast(x0_v[...], BF16)
                qkv0_vs[i][h] = _dot(x0, wblk(i, h)).astype(BF16)
                if i < 2:
                    relayout(i + 1, h)
                else:
                    wo_pack(h)
            return c
        jax.lax.fori_loop(0, 4, bbody, 0)

    x_v[0, 0:M, :] = mem0_v[...]
    for j in range(2 * HB):
        lk_v[j * NSEG * M:j * NSEG * M + 64, :] = jnp.zeros((64, DHB), BF16)

    def qk_chunk(u, slot, c, mx, gate=None):
        st = _dot(ka_v[c * CH:(c + 1) * CH, :], qt_v[u])
        st_v[slot, c * CH:(c + 1) * CH, :] = st
        cm = jnp.max(st.reshape(CH // 8, 8, 512), axis=0)
        if gate is not None:
            for r in range(0, CH, 64):
                gate(st[r:r + 8, 0:128])
        return cm if mx is None else jnp.maximum(mx, cm)

    PR = CH // NPC

    def pv_exp(slot, r, m8):
        st = st_v[slot, r:r + PR, :].reshape(PR // 8, 8, 512)
        p = jnp.exp2(st - m8[None])
        pk = p.reshape(PR, 512).astype(BF16)
        while p.shape[0] > 1:
            p = p.reshape(p.shape[0] // 2, 2, 8, 512)
            p = p[:, 0] + p[:, 1]
        return p[0], pk

    def colmax(mx):
        return jnp.broadcast_to(jnp.max(mx, axis=0, keepdims=True), (8, 512))

    def a_finish(u, l, acc):
        o = acc * _recip(jnp.sum(l, axis=0, keepdims=True))
        o4 = jnp.concatenate([o[:, j * 128:(j + 1) * 128] for j in range(4)], axis=0)
        qb = u // 8
        b = u % 8
        oa_v[pl.ds(pl.multiple_of(qb * 128, 128), 128),
             pl.ds(pl.multiple_of(b * 128, 128), 128)] = o4.T.astype(BF16)

    mxs = [None, None]
    for n in range(QL):
        t, c = divmod(n, NCH)
        mxs[t] = qk_chunk(t, t, c, mxs[t])
    mx_v[0] = mxs[0]
    mx_v[1] = mxs[1]
    fin_v[...] = jnp.ones((40, 512), F32)

    bscale = DHB ** -0.5
    ri = jax.lax.broadcasted_iota(jnp.int32, (SEG, L), 0)
    ci = jax.lax.broadcasted_iota(jnp.int32, (SEG, L), 1)
    mask = (ri < M) | (ci >= SEG) | (ri >= ci)
    gr = jax.lax.broadcasted_iota(jnp.int32, (64, 128), 0)
    gc = jax.lax.broadcasted_iota(jnp.int32, (64, 128), 1)
    gsame = (gr // M) == ((gc % 64) // M)
    gmask = gsame & ((gc < 64) | (gr >= gc - 64))

    def softmax_nonorm(sc):
        p = jnp.exp(sc - jnp.max(sc, axis=1, keepdims=True))
        return p.astype(BF16), _recip(jnp.sum(p, axis=1, keepdims=True))

    def grp_qk(grp, hd):
        rs = pl.ds(pl.multiple_of(grp * 64, 64), 64)
        k = jnp.concatenate([lk_v[kvm_rows(0, hd, grp * 64, 64), :], k0_v[hd, rs, :]], axis=0)
        sc = _dot_nt(q0_v[hd, rs, :], k) * bscale
        sc = jnp.where(gmask, sc, jnp.where(gsame, NEG, -jnp.inf))
        return softmax_nonorm(sc)

    def grp_pv(grp, hd, pr, last=False):
        rs = pl.ds(pl.multiple_of(grp * 64, 64), 64)
        v = jnp.concatenate([lk_v[kvm_rows(1, hd, grp * 64, 64), :], v0_v[hd, rs, :]], axis=0)
        o = (_dot(pr[0], v) * pr[1]).astype(BF16)
        cs = pl.ds(pl.multiple_of(hd * 128, 128), 128)
        if last:
            o7_v[:, cs] = o
        else:
            o0_v[rs, cs] = o

    NP = HB // 2
    item_gate = []
    ng = 0
    for k in range(NP + 2):
        ng += 6 if k < NP else 0
        if k in A_AFTER_PART:
            item_gate.append(ng)
            ng += 4
    for c in range(8):
        ng += WOS
        if c in A_AFTER_WO:
            item_gate.append(ng)
            ng += 4
    while len(item_gate) < NIT:
        item_gate.append(ng)
        ng += 4
    plan = {}
    for k in range(NIT * NPC):
        n = k // NPC
        lo = 0 if n < NCH else item_gate[2 * NCH - 1 - QL] + 4
        g = max(lo, k * ng // (NIT * NPC) - LEAD)
        g = max(lo, min(g, item_gate[n] - MARGIN))
        plan.setdefault(g, []).append(k)

    def step(s, carry):
        h = x_v[s]
        r0 = pl.multiple_of(s * M, M)
        grp = jnp.maximum(s // 8 - 1, 0)
        gh0 = (s % 8) * 4

        mx = {0: mx_v[0], 1: mx_v[1]}
        m8 = {0: colmax(mx[0])}
        ls = {}
        acc = {}
        pks = {}
        gates = [0]

        def gate(dep):
            for k in plan.get(gates[0], ()):
                n, i = divmod(k, NPC)
                t, c = divmod(n, NCH)
                dep4 = jnp.concatenate([dep] * 4, axis=1)
                m = jnp.where(dep4 > jnp.inf, dep4, m8[t])
                cl, pk = pv_exp(t % 2, c * CH + i * PR, m)
                pks.setdefault(n, []).append(pk)
                ls[t] = cl if t not in ls else ls[t] + cl
            gates[0] += 1

        def a_item(j):
            t, c = divmod(j + QL, NCH)
            u = jnp.minimum(s * 2 + t, NUNIT - 1)
            mx[t] = qk_chunk(u, t % 2, c, mx.get(t), gate)
            if c == NCH - 1:
                m8[t] = colmax(mx[t])
            t, c = divmod(j, NCH)
            o = _dot(vt_v[:, c * CH:(c + 1) * CH], jnp.concatenate(pks.pop(j), axis=0))
            acc[t] = o if t not in acc else acc[t] + o
            if j == NCH - 1:
                a_finish(s * 2, ls[0], acc[0])

        def proj(hd):
            qkv = []
            for i in range(3):
                y = _dot(h, wblk(i, hd))
                gate(y[0:8])
                qkv.append(y.astype(BF16))
            q, k, v = qkv
            lk_v[kvm_rows(0, hd, r0, M), :] = k[:M]
            lk_v[kvm_rows(1, hd, r0, M), :] = v[:M]
            return q, k, v

        def attn_qk(hd, qkv):
            q, k, v = qkv
            k = jnp.concatenate([k, k0_v[hd, pl.ds(r0, M), :]], axis=0)
            v = jnp.concatenate([v, v0_v[hd, pl.ds(r0, M), :]], axis=0)
            sc = jnp.where(mask, _dot_nt(q, k) * bscale, NEG)
            return softmax_nonorm(sc) + (v,)

        def attn_pv(hd, prv):
            p, r, v = prv
            o = (_dot(p, v) * r).astype(BF16)
            ocat_v[:, hd * 128:(hd + 1) * 128] = pltpu.bitcast(o, U32)

        def g_work(k):
            for j in range(4):
                if GP_AFTER_PART[j] == k:
                    grp_pv(grp, gh0 + j, gps.pop(j))
            for j in range(4):
                if GQ_AFTER_PART[j] == k:
                    gps[j] = grp_qk(grp, gh0 + j)

        a_finish(jnp.maximum(s * 2 - 1, 0), fin_v[32:40, :], fin_v[0:32, :])
        projs = {}
        pvs = {}
        gps = {}
        g_work(-1)
        na = 0
        for k in range(NP + 2):
            if k < NP:
                for j in range(2):
                    projs[2 * k + j] = proj(2 * k + j)
            if k >= 2:
                for j in range(2):
                    hd = 2 * (k - 2) + j
                    attn_pv(hd, pvs.pop(hd))
            if 1 <= k <= NP:
                for j in range(2):
                    hd = 2 * (k - 1) + j
                    pvs[hd] = attn_qk(hd, projs.pop(hd))
            g_work(k)
            if k in A_AFTER_PART:
                a_item(na)
                na += 1
        ys = []
        KW = HB * DHB // WOS
        for c in range(8):
            y = None
            for w in range(WOS):
                oc = pltpu.bitcast(ocat_v[:, w * KW:(w + 1) * KW], BF16)
                wo = pltpu.bitcast(
                    wo_v[c * 2048 + w * KW // 2:c * 2048 + (w + 1) * KW // 2, :], BF16)
                yw = _dot(oc, wo)
                gate(yw[0:8])
                y = yw if y is None else y + yw
            ys.append(y)
            g_work(20 + c)
            if c in A_AFTER_WO:
                a_item(na)
                na += 1
        y = jnp.concatenate(ys, axis=1)
        b_v[s, M:, :] = y[M:]
        x_v[jnp.minimum(s + 1, NSEG - 1), 0:M, :] = y[:M].astype(BF16)
        while na < NIT:
            a_item(na)
            na += 1
        mx_v[0] = mx[2]
        mx_v[1] = mx[3]
        fin_v[0:32, :] = acc[1]
        fin_v[32:40, :] = ls[1]
        return carry

    jax.lax.fori_loop(0, NSTEPS, step, 0, unroll=UNROLL)

    a_finish(NUNIT - 1, fin_v[32:40, :], fin_v[0:32, :])
    woa_copy.wait()
    EB = 256
    NEB = S // EB

    def out_copy(i):
        return pltpu.make_async_copy(x_v.at[pl.ds(i * 8, 8)],
                                     out_hbm.at[pl.ds(i * 8, 8)], sem_out.at[i])

    def eblock(i, nlast):
        r0 = pl.multiple_of(i * EB, EB)
        s0 = pl.multiple_of(i * 8, 8)
        o0 = o0_v[pl.ds(pl.multiple_of(i * 64, 64), 64), :]
        oa = oa_v[pl.ds(r0, EB), :]
        gps = {}
        for c in range(8):
            cs = slice(c * 128, (c + 1) * 128)
            b0 = _dot(o0, woblk(c)).reshape(8, M, 128)
            b = jnp.concatenate([b0, b_v[pl.ds(s0, 8), M:, cs]], axis=1).reshape(EB, 128)
            if nlast and 1 <= c <= 4:
                for j in (2 * c - 2, 2 * c - 1):
                    grp_pv(7, i * 8 + j, gps.pop(j), True)
            a = _dot(oa, woa_v[:, cs])
            g = g_v[pl.ds(r0, EB), :]
            x_v[pl.ds(s0, 8), :, cs] = (
                g * a + (1.0 - g) * b).astype(BF16).reshape(8, SEG, 128)
            if nlast and c < 4:
                for j in (2 * c, 2 * c + 1):
                    gps[j] = grp_qk(7, i * 8 + j)
        out_copy(i).start()

    def ebody0(i, carry):
        eblock(i, 8)
        return carry

    def ebody1(i, carry):
        eblock(i, 0)
        return carry
    jax.lax.fori_loop(0, 4, ebody0, 0)
    o0_v[pl.ds(7 * 64, 64), :] = o7_v[...]
    jax.lax.fori_loop(4, NEB, ebody1, 0)
    for i in range(NEB):
        out_copy(i).wait()


@functools.partial(jax.jit, static_argnames=("B_seg_len",))
def pallas_gated_mix__grouped_kv_mqa__memory_aug_recurrent_mem_tr__prompt_kernel(
    A_x, A_wq, A_wk, A_wv, A_wo, B_x, B_mem0, B_Wq, B_Wk, B_Wv, B_Wo, B_seg_len,
    gate_w,
):
    del B_x
    assert B_seg_len == SEG and A_x.shape == (1, S, D)
    hbm = pl.BlockSpec(memory_space=pl.ANY)
    wsc = pltpu.VMEM((HB, D // 2, DHB), U32)
    p0sc = pltpu.VMEM((HB, NSEG * M, DHB), BF16)
    lsc = pltpu.VMEM((D * HB, DHB), BF16)
    out = pl.pallas_call(
        _kernel,
        out_shape=jax.ShapeDtypeStruct((NSEG, SEG, D), BF16),
        in_specs=[hbm] * 11,
        out_specs=hbm,
        scratch_shapes=[
            pltpu.VMEM((NSEG, SEG, D), BF16),
            pltpu.VMEM((NSEG * M // 2, D), U32),
            pltpu.VMEM((D, D), BF16),
            pltpu.VMEM((D, D), BF16),
            pltpu.VMEM((80, D), BF16),
            pltpu.VMEM((8, 128), BF16),
            pltpu.VMEM((M, D), BF16),
            wsc, wsc, wsc,
            pltpu.VMEM((8 * HB * DHB // 2, 128), U32),
            pltpu.VMEM((NUNIT, DHA, 512), BF16),
            pltpu.VMEM((S, DHA), BF16),
            pltpu.VMEM((DHA, S), BF16),
            pltpu.VMEM((S, 128), F32),
            p0sc, p0sc, p0sc,
            lsc, lsc, lsc,
            pltpu.VMEM((800, 128), U32),
            pltpu.VMEM((800, 128), U32),
            pltpu.VMEM((2, S, 512), F32),
            pltpu.VMEM((2, 8, 512), F32),
            pltpu.VMEM((40, 512), F32),
            pltpu.VMEM((SEG // 2, HB * DHB), U32),
            pltpu.VMEM((NSEG * M, HB * DHB), BF16),
            pltpu.VMEM((64, HB * DHB), BF16),
            pltpu.VMEM((NSEG, SEG, D), F32),
            pltpu.VMEM((S, D), BF16),
            pltpu.SemaphoreType.DMA((4,)),
            pltpu.SemaphoreType.DMA((4,)),
            pltpu.SemaphoreType.DMA((5,)),
            pltpu.SemaphoreType.DMA((4,)),
            pltpu.SemaphoreType.DMA((8,)),
            pltpu.SemaphoreType.DMA((8,)),
        ],
        compiler_params=pltpu.CompilerParams(vmem_limit_bytes=127 * 1024 * 1024),
    )(
        A_x.reshape(NSEG, SEG, D), A_wq, A_wk.T, A_wv.T, A_wo, B_mem0.reshape(M, D),
        B_Wq.reshape(D * HB, DHB), B_Wk.reshape(D * HB, DHB),
        B_Wv.reshape(D * HB, DHB), B_Wo.reshape(HB * DHB, D),
        gate_w.reshape(8, 128),
    )
    return out.reshape(1, S, D)
```

```python
import functools
import math

import jax
import jax.numpy as jnp
import jax.experimental.pallas as pl
import jax.experimental.pallas.tpu as pltpu

F32 = jnp.float32
BF16 = jnp.bfloat16
U32 = jnp.uint32

S = 2048
D = 1024
DHA = 32
HB = 32
DHB = 128
M = 8
SEG = 32
NSEG = S // SEG
L = M + SEG
NUNIT = (S // 128) * (D // 128)
CH = 256
NCH = S // CH
NIT = 2 * NCH
NT = (((1,), (1,)), ((), ()))
NEG = -1000000000.0
NSTEPS = NSEG
A_AFTER_PART = [1,3,4,6,7,9,10,12,13,15,16,17]
A_AFTER_WO = [1,4,6]
GQ_AFTER_PART = [17,21,23,25]
GP_AFTER_PART = [21,23,25,27]
QL = 10
WQC = 2
DM = 1
NPC = 8
MARGIN = 1
LEAD = 12
WOS = 4
UNROLL = 2
BH = 8
BH2 = 8
PAD = 0
FB = 2
G0 = 0
G1 = 256
GS = 32
FINE = 1
MDEP = 1


def _dot(a, b):
    return jnp.dot(a, b, preferred_element_type=F32)


def _dot_nt(a, b):
    return jax.lax.dot_general(a, b, NT, preferred_element_type=F32)


def _recip(x):
    return pl.reciprocal(x, approx=False, full_range=False)


def _kernel(x_hbm, wqa_hbm, wka_hbm, wva_hbm, woa_hbm, mem0_hbm, wq_hbm, wk_hbm,
            wv_hbm, wo_hbm, gw_hbm, out_hbm,
            x_v, x0_v, wqa_v, woa_v, wkvz_v, gw_v, mem0_v, w_v, wo_v,
            qt_v, ka_v, vt_v, g_v, p0_v, land_v,
            sg0_v, sg1_v, st_v, mx_v, fin_v, ocat_v, o0_v, o7_v, b_v, oa_v,
            sem_x, sem_s, sem_wa, sem_w, sem_wo, sem_out):
    XCH = ((0, FB), (FB, 6), (6, 8), (8, 12), (12, 16))
    w_hbms = (wq_hbm, wk_hbm, wv_hbm)
    WR = D * HB
    stg_vs = (sg0_v, sg1_v)

    def x_copy(i):
        rs = pl.ds(4 * XCH[i][0], 4 * (XCH[i][1] - XCH[i][0]))
        return pltpu.make_async_copy(x_hbm.at[rs], x_v.at[rs], sem_x.at[i])

    small = [
        pltpu.make_async_copy(wka_hbm, wkvz_v.at[pl.ds(0, DHA)], sem_s.at[0]),
        pltpu.make_async_copy(wva_hbm, wkvz_v.at[pl.ds(DHA, DHA)], sem_s.at[1]),
        pltpu.make_async_copy(gw_hbm, gw_v, sem_s.at[2]),
        pltpu.make_async_copy(mem0_hbm, mem0_v, sem_s.at[3]),
    ]

    def wqa_copy(c):
        cs = pl.ds(c * (D // WQC), D // WQC)
        return pltpu.make_async_copy(wqa_hbm.at[:, cs], wqa_v.at[:, cs], sem_wa.at[c])

    woa_copy = pltpu.make_async_copy(woa_hbm, woa_v, sem_wa.at[4])

    def w_copy(i, j):
        return pltpu.make_async_copy(
            w_hbms[i].at[pl.ds(j * (WR // 2), WR // 2)],
            land_v.at[pl.ds((2 * i + j) * (WR // 2), WR // 2)], sem_w.at[2 * i + j])

    def w_wait(n):
        pltpu.make_async_copy(
            wq_hbm.at[pl.ds(0, WR // 2)],
            land_v.at[pl.ds(pl.multiple_of(n * (WR // 2), WR // 2), WR // 2)],
            sem_w.at[n]).wait()

    def wo_copy(c):
        return pltpu.make_async_copy(wo_hbm.at[:, pl.ds(c * 128, 128)],
                                     land_v.at[pl.ds(c * HB * DHB, HB * DHB)],
                                     sem_wo.at[c])

    x_copy(0).start()
    for cp in small:
        cp.start()
    for c in range(WQC):
        wqa_copy(c).start()

    def kvm_rows(kv, hd, r, n):
        return pl.ds(pl.multiple_of(WR + (kv * HB + hd) * (NSEG * M) + r, M), n)

    qscale = (DHA ** -0.5) * math.log2(math.e)

    def xblk(rb):
        return x_v[pl.ds(rb * 4, 4)].reshape(128, D)

    def aproj_kvz(rb):
        kvz = _dot_nt(wkvz_v[...], xblk(rb))
        r0 = pl.multiple_of(rb * 128, 128)
        vt_v[:, pl.ds(r0, 128)] = kvz[DHA:2 * DHA, :].astype(BF16)
        t = jnp.concatenate([kvz, jnp.zeros((48, 128), F32)], axis=0).T
        ka_v[pl.ds(r0, 128), :] = t[:, :DHA].astype(BF16)
        x0 = x_v[pl.ds(rb * 4, 4), 0:M, :].reshape(4 * M, D)
        x0_v[pl.ds(pl.multiple_of(rb * 16, 16), 16), :] = pltpu.bitcast(x0, U32)
        g_v[pl.ds(r0, 128), :] = jnp.broadcast_to(
            jax.nn.sigmoid(t[:, 2 * DHA:2 * DHA + 1]), (128, 128))

    def aproj_q(rb, b):
        q = _dot(xblk(rb), wqa_v[:, b * 128:(b + 1) * 128]) * qscale
        qT = q.T.astype(BF16)
        for j in range(4):
            qt_v[rb * 8 + b, :, j * 128:(j + 1) * 128] = qT[j * 32:(j + 1) * 32, :]
        return [q[16 * k:16 * k + 16] for k in range(8)] if FINE else q[0:16]

    def aproj(rb, extra=()):
        extra = list(extra)
        aproj_kvz(rb)
        for b in range(8):
            dep = aproj_q(rb, b)
            if extra:
                extra.pop(0)(dep=dep)

    def relayout(i, g, blks=(0, 1), dep=None):
        for blk in blks:
            stg = stg_vs[blk]
            base = pl.multiple_of(i * WR + g * 1024 + blk * 512, 512)
            v = pltpu.bitcast(land_v[pl.ds(base, 512), :], U32)
            for k in range(8):
                a = v[32 * k:32 * k + 16]
                b = v[32 * k + 16:32 * k + 32]
                if dep is not None:
                    dk = dep[k] if isinstance(dep, list) else dep
                    a = jnp.where(dk > jnp.inf, U32(0), a)
                stg[pl.ds(3 * k, 16, stride=25), :] = (a & U32(0xffff)) | (b << 16)
                stg[pl.ds(400 + 3 * k, 16, stride=25), :] = (a >> 16) | (b & U32(0xffff0000))
            r = pl.multiple_of(g * 16 + blk * 8, 8)
            for p in range(16):
                w_v[i, 2 * p, pl.ds(r, 8), :] = stg[pl.ds(25 * p, 8, stride=3), :]
                w_v[i, 2 * p + 1, pl.ds(r, 8), :] = stg[pl.ds(400 + 25 * p, 8, stride=3), :]

    def wo_pack(g):
        v = land_v[pl.ds(pl.multiple_of(g * 1024, 1024), 1024), :]
        wo_v[pl.ds(pl.multiple_of(g * 512, 512), 512), :] = pltpu.bitcast(v, U32)

    def wblk(i, h):
        return pltpu.bitcast(w_v[i, h], BF16)

    def woblk(c):
        return pltpu.bitcast(wo_v[c * 2048:(c + 1) * 2048, :], BF16)

    for cp in small:
        cp.wait()
    gw = gw_v[...]
    gw_row = jnp.concatenate([gw[r:r + 1, :] for r in range(8)], axis=1)
    wkvz_v[2 * DHA:, :] = jnp.broadcast_to(gw_row, (16, D))
    x_copy(0).wait()
    for i in range(1, len(XCH)):
        x_copy(i).start()
    for i in range(2):
        for j in range(2):
            w_copy(i, j).start()
    for rb in range(FB):
        aproj_kvz(rb)
    for c in range(WQC):
        wqa_copy(c).wait()
        for rb in range(FB):
            for b in range(c * (8 // WQC), (c + 1) * (8 // WQC)):
                aproj_q(rb, b)
    x_copy(1).wait()

    def abody0(t, c):
        @pl.when(t == 3)
        def _():
            x_copy(2).wait()
        aproj(t * 2)
        aproj(t * 2 + 1)
        return c
    jax.lax.fori_loop(FB // 2, 4, abody0, 0)
    x_copy(3).wait()
    w_copy(0, 0).wait()

    def abody1(t, c):
        @pl.when(t == 2)
        def _():
            x_copy(4).wait()
            w_copy(0, 1).wait()
            w_copy(2, 0).start()
            w_copy(2, 1).start()
        for k in range(2):
            g0 = t * 8 + k * 4
            aproj(8 + t * 2 + k,
                  [functools.partial(relayout, 0, g0 + r // 2, (r % 2,))
                   for r in range(8)])
        return c
    jax.lax.fori_loop(0, 4, abody1, 0)

    def qk_chunk(u, slot, c, mx, gate=None):
        rs = pl.ds(c * CH, CH) if isinstance(c, int) else pl.ds(pl.multiple_of(c * CH, CH), CH)
        st = _dot(ka_v[rs, :], qt_v[u])
        st_v[slot, rs, :] = st
        cm = jnp.max(st.reshape(CH // 8, 8, 512), axis=0)
        if gate is not None:
            for r in range(0, CH, 64):
                gate(st[r:r + 8, 0:128])
        return cm if mx is None else jnp.maximum(mx, cm)

    for c in range(8):
        wo_copy(c).start()
    woa_copy.start()

    def bulk(i, h):
        x0 = pltpu.bitcast(x0_v[...], BF16)
        y = _dot(x0, wblk(i, h))
        p0_v[i, h] = y.astype(BF16)
        return y

    def bbody0(n, c):
        @pl.when(n % 2 == 0)
        def _():
            w_wait(2 + n // 2)
        y = None
        for hh in range(8):
            h = (n % 4) * 8 + hh
            deps = (None, None) if y is None else [
                [y[G0 + b * G1 + k * GS:G0 + b * G1 + k * GS + 16] for k in range(8)]
                for b in range(2)]
            y = bulk(n // 4, h)
            for blk in range(2):
                relayout(n // 4 + 1, h, (blk,), deps[blk])
        return c
    jax.lax.fori_loop(0, 8, bbody0, 0)
    for c in range(8):
        wo_copy(c).wait()
    mx_v[0] = jnp.full((8, 512), -jnp.inf, F32)

    def bbody1(n, c):
        for hh in range(4):
            bulk(2, n * 4 + hh)
            wo_pack(n * 4 + hh)
            if hh == 1:
                mx_v[0] = qk_chunk(0, 0, n, mx_v[0])
        return c
    jax.lax.fori_loop(0, 8, bbody1, 0)

    x_v[0, 0:M, :] = mem0_v[...]
    for j in range(2 * HB):
        land_v[WR + j * NSEG * M:WR + j * NSEG * M + 64, :] = jnp.zeros((64, DHB), BF16)

    PR = CH // NPC

    def pv_exp(slot, r, m8):
        st = st_v[slot, r:r + PR, :].reshape(PR // 8, 8, 512)
        p = jnp.exp2(st - m8[None])
        pk = p.reshape(PR, 512).astype(BF16)
        while p.shape[0] > 1:
            p = p.reshape(p.shape[0] // 2, 2, 8, 512)
            p = p[:, 0] + p[:, 1]
        return p[0], pk

    def colmax(mx):
        return jnp.broadcast_to(jnp.max(mx, axis=0, keepdims=True), (8, 512))

    def a_finish(u, l, acc):
        o = acc * _recip(jnp.sum(l, axis=0, keepdims=True))
        o4 = jnp.concatenate([o[:, j * 128:(j + 1) * 128] for j in range(4)], axis=0)
        qb = u // 8
        b = u % 8
        oa_v[pl.ds(pl.multiple_of(qb * 128, 128), 128),
             pl.ds(pl.multiple_of(b * 128, 128), 128)] = o4.T.astype(BF16)

    mx1 = None
    for c in range(QL - NCH):
        mx1 = qk_chunk(1, 1, c, mx1)
    mx_v[1] = mx1
    fin_v[...] = jnp.ones((40, 512), F32)

    bscale = DHB ** -0.5
    ri = jax.lax.broadcasted_iota(jnp.int32, (SEG, L), 0)
    ci = jax.lax.broadcasted_iota(jnp.int32, (SEG, L), 1)
    mask = (ri < M) | (ci >= SEG) | (ri >= ci)
    gr = jax.lax.broadcasted_iota(jnp.int32, (64, 128), 0)
    gc = jax.lax.broadcasted_iota(jnp.int32, (64, 128), 1)
    gsame = (gr // M) == ((gc % 64) // M)
    gmask = gsame & ((gc < 64) | (gr >= gc - 64))

    def softmax_nonorm(sc):
        p = jnp.exp(sc - jnp.max(sc, axis=1, keepdims=True))
        return p.astype(BF16), _recip(jnp.sum(p, axis=1, keepdims=True))

    def grp_qk(grp, hd):
        rs = pl.ds(pl.multiple_of(grp * 64, 64), 64)
        k = jnp.concatenate([land_v[kvm_rows(0, hd, grp * 64, 64), :], p0_v[1, hd, rs, :]], axis=0)
        sc = _dot_nt(p0_v[0, hd, rs, :], k) * bscale
        sc = jnp.where(gmask, sc, jnp.where(gsame, NEG, -jnp.inf))
        return softmax_nonorm(sc)

    def grp_pv(grp, hd, pr, last=False):
        rs = pl.ds(pl.multiple_of(grp * 64, 64), 64)
        v = jnp.concatenate([land_v[kvm_rows(1, hd, grp * 64, 64), :], p0_v[2, hd, rs, :]], axis=0)
        o = (_dot(pr[0], v) * pr[1]).astype(BF16)
        cs = pl.ds(pl.multiple_of(hd * 128, 128), 128)
        if last:
            o7_v[:, cs] = o
        else:
            o0_v[rs, cs] = o

    NP = HB // 2
    item_gate = []
    ng = 0
    for k in range(NP + 2):
        ng += 6 if k < NP else 0
        if k in A_AFTER_PART:
            item_gate.append(ng)
            ng += 4
    for c in range(8):
        ng += WOS
        if c in A_AFTER_WO:
            item_gate.append(ng)
            ng += 4
    while len(item_gate) < NIT:
        item_gate.append(ng)
        ng += 4
    plan = {}
    for k in range(NIT * NPC):
        n = k // NPC
        lo = 0 if n < NCH else item_gate[2 * NCH - 1 - QL] + 4
        g = max(lo, k * ng // (NIT * NPC) - LEAD)
        g = max(lo, min(g, item_gate[n] - MARGIN))
        plan.setdefault(g, []).append(k)

    def step(s, carry):
        h = x_v[s]
        r0 = pl.multiple_of(s * M, M)
        grp = jnp.maximum(s // 8 - 1, 0)
        gh0 = (s % 8) * 4

        mx = {0: mx_v[0], 1: mx_v[1]}
        m8 = {0: colmax(mx[0])}
        ls = {}
        acc = {}
        pks = {}
        gates = [0]

        def gate(dep):
            for k in plan.get(gates[0], ()):
                n, i = divmod(k, NPC)
                t, c = divmod(n, NCH)
                dep4 = jnp.concatenate([dep] * 4, axis=1)
                m = jnp.where(dep4 > jnp.inf, dep4, m8[t])
                cl, pk = pv_exp(t % 2, c * CH + i * PR, m)
                pks.setdefault(n, []).append(pk)
                ls[t] = cl if t not in ls else ls[t] + cl
            gates[0] += 1

        def a_item(j):
            t, c = divmod(j + QL, NCH)
            u = jnp.minimum(s * 2 + t, NUNIT - 1)
            mx[t] = qk_chunk(u, t % 2, c, mx.get(t), gate)
            if c == NCH - 1:
                m8[t] = colmax(mx[t])
            t, c = divmod(j, NCH)
            o = _dot(vt_v[:, c * CH:(c + 1) * CH], jnp.concatenate(pks.pop(j), axis=0))
            acc[t] = o if t not in acc else acc[t] + o
            if j == NCH - 1:
                a_finish(s * 2, ls[0], acc[0])

        def proj(hd):
            qkv = []
            for i in range(3):
                y = _dot(h, wblk(i, hd))
                gate(y[0:8])
                qkv.append(y.astype(BF16))
            q, k, v = qkv
            land_v[kvm_rows(0, hd, r0, M), :] = k[:M]
            land_v[kvm_rows(1, hd, r0, M), :] = v[:M]
            return q, k, v

        def attn_qk(hd, qkv):
            q, k, v = qkv
            k = jnp.concatenate([k, p0_v[1, hd, pl.ds(r0, M), :]], axis=0)
            v = jnp.concatenate([v, p0_v[2, hd, pl.ds(r0, M), :]], axis=0)
            sc = jnp.where(mask, _dot_nt(q, k) * bscale, NEG)
            return softmax_nonorm(sc) + (v,)

        def attn_pv(hd, prv):
            p, r, v = prv
            o = (_dot(p, v) * r).astype(BF16)
            ocat_v[:, hd * 128:(hd + 1) * 128] = pltpu.bitcast(o, U32)

        def g_work(k):
            for j in range(4):
                if GP_AFTER_PART[j] == k:
                    grp_pv(grp, gh0 + j, gps.pop(j))
            for j in range(4):
                if GQ_AFTER_PART[j] == k:
                    gps[j] = grp_qk(grp, gh0 + j)

        a_finish(jnp.maximum(s * 2 - 1, 0), fin_v[32:40, :], fin_v[0:32, :])
        projs = {}
        pvs = {}
        gps = {}
        g_work(-1)
        na = 0
        for k in range(NP + 2):
            if k < NP:
                for j in range(2):
                    projs[2 * k + j] = proj(2 * k + j)
            if k >= 2:
                for j in range(2):
                    hd = 2 * (k - 2) + j
                    attn_pv(hd, pvs.pop(hd))
            if 1 <= k <= NP:
                for j in range(2):
                    hd = 2 * (k - 1) + j
                    pvs[hd] = attn_qk(hd, projs.pop(hd))
            g_work(k)
            if k in A_AFTER_PART:
                a_item(na)
                na += 1
        ys = []
        KW = HB * DHB // WOS
        for c in range(8):
            y = None
            for w in range(WOS):
                oc = pltpu.bitcast(ocat_v[:, w * KW:(w + 1) * KW], BF16)
                wo = pltpu.bitcast(
                    wo_v[c * 2048 + w * KW // 2:c * 2048 + (w + 1) * KW // 2, :], BF16)
                yw = _dot(oc, wo)
                gate(yw[0:8])
                y = yw if y is None else y + yw
            ys.append(y)
            g_work(20 + c)
            if c in A_AFTER_WO:
                a_item(na)
                na += 1
        y = jnp.concatenate(ys, axis=1)
        b_v[s, M:, :] = y[M:]
        x_v[jnp.minimum(s + 1, NSEG - 1), 0:M, :] = y[:M].astype(BF16)
        while na < NIT:
            a_item(na)
            na += 1
        mx_v[0] = mx[2]
        mx_v[1] = mx[3]
        fin_v[0:32, :] = acc[1]
        fin_v[32:40, :] = ls[1]
        return carry

    jax.lax.fori_loop(0, NSTEPS, step, 0, unroll=UNROLL)

    a_finish(NUNIT - 1, fin_v[32:40, :], fin_v[0:32, :])
    woa_copy.wait()
    EB = 256
    NEB = S // EB

    def out_copy(i):
        return pltpu.make_async_copy(x_v.at[pl.ds(i * 8, 8)],
                                     out_hbm.at[pl.ds(i * 8, 8)], sem_out.at[i])

    def eblock(i, carry):
        r0 = pl.multiple_of(i * EB, EB)
        s0 = pl.multiple_of(i * 8, 8)
        o0 = o0_v[pl.ds(pl.multiple_of(i * 64, 64), 64), :]
        oa = oa_v[pl.ds(r0, EB), :]
        gps = {}
        hds = [jnp.minimum(i * 5 + j, HB - 1) for j in range(5)]
        for c in range(8):
            cs = slice(c * 128, (c + 1) * 128)
            b0 = _dot(o0, woblk(c)).reshape(8, M, 128)
            b = jnp.concatenate([b0, b_v[pl.ds(s0, 8), M:, cs]], axis=1).reshape(EB, 128)
            if 1 <= c <= 5:
                grp_pv(7, hds[c - 1], gps.pop(c - 1), True)
            a = _dot(oa, woa_v[:, cs])
            g = g_v[pl.ds(r0, EB), :]
            x_v[pl.ds(s0, 8), :, cs] = (
                g * a + (1.0 - g) * b).astype(BF16).reshape(8, SEG, 128)
            if c < 5:
                gps[c] = grp_qk(7, hds[c])
        out_copy(i).start()

        @pl.when(i == NEB - 2)
        def _():
            o0_v[pl.ds(7 * 64, 64), :] = o7_v[...]
        return carry

    jax.lax.fori_loop(0, NEB, eblock, 0)
    for i in range(NEB):
        out_copy(i).wait()


@functools.partial(jax.jit, static_argnames=("B_seg_len",))
def pallas_gated_mix__grouped_kv_mqa__memory_aug_recurrent_mem_tr__prompt_kernel(
    A_x, A_wq, A_wk, A_wv, A_wo, B_x, B_mem0, B_Wq, B_Wk, B_Wv, B_Wo, B_seg_len,
    gate_w,
):
    del B_x
    assert B_seg_len == SEG and A_x.shape == (1, S, D)
    hbm = pl.BlockSpec(memory_space=pl.ANY)
    out = pl.pallas_call(
        _kernel,
        out_shape=jax.ShapeDtypeStruct((NSEG, SEG, D), BF16),
        in_specs=[hbm] * 11,
        out_specs=hbm,
        scratch_shapes=[
            pltpu.VMEM((NSEG, SEG, D), BF16),
            pltpu.VMEM((NSEG * M // 2, D), U32),
            pltpu.VMEM((D, D), BF16),
            pltpu.VMEM((D, D), BF16),
            pltpu.VMEM((80, D), BF16),
            pltpu.VMEM((8, 128), BF16),
            pltpu.VMEM((M, D), BF16),
            pltpu.VMEM((3, HB, D // 2, DHB), U32),
            pltpu.VMEM((8 * HB * DHB // 2, 128), U32),
            pltpu.VMEM((NUNIT, DHA, 512), BF16),
            pltpu.VMEM((S, DHA), BF16),
            pltpu.VMEM((DHA, S), BF16),
            pltpu.VMEM((S, 128), F32),
            pltpu.VMEM((3, HB, NSEG * M, DHB), BF16),
            pltpu.VMEM((3 * D * HB, DHB), BF16),
            pltpu.VMEM((832, 128), U32),
            pltpu.VMEM((832, 128), U32),
            pltpu.VMEM((2, S, 512), F32),
            pltpu.VMEM((2, 8, 512), F32),
            pltpu.VMEM((40, 512), F32),
            pltpu.VMEM((SEG // 2, HB * DHB), U32),
            pltpu.VMEM((NSEG * M, HB * DHB), BF16),
            pltpu.VMEM((64, HB * DHB), BF16),
            pltpu.VMEM((NSEG, SEG, D), F32),
            pltpu.VMEM((S, D), BF16),
            pltpu.SemaphoreType.DMA((5,)),
            pltpu.SemaphoreType.DMA((4,)),
            pltpu.SemaphoreType.DMA((5,)),
            pltpu.SemaphoreType.DMA((6,)),
            pltpu.SemaphoreType.DMA((8,)),
            pltpu.SemaphoreType.DMA((8,)),
        ],
        compiler_params=pltpu.CompilerParams(vmem_limit_bytes=127 * 1024 * 1024),
    )(
        A_x.reshape(NSEG, SEG, D), A_wq, A_wk.T, A_wv.T, A_wo, B_mem0.reshape(M, D),
        B_Wq.reshape(D * HB, DHB), B_Wk.reshape(D * HB, DHB),
        B_Wv.reshape(D * HB, DHB), B_Wo.reshape(HB * DHB, D),
        gate_w.reshape(8, 128),
    )
    return out.reshape(1, S, D)
```

```python
import functools
import math

import jax
import jax.numpy as jnp
import jax.experimental.pallas as pl
import jax.experimental.pallas.tpu as pltpu

F32 = jnp.float32
BF16 = jnp.bfloat16
U32 = jnp.uint32

S = 2048
D = 1024
DHA = 32
HB = 32
DHB = 128
M = 8
SEG = 32
NSEG = S // SEG
L = M + SEG
NUNIT = (S // 128) * (D // 128)
CH = 256
NCH = S // CH
NIT = 2 * NCH
NPC = 8
PR = CH // NPC
QL = 10
LEAD = 12
WOS = 4
NT = (((1,), (1,)), ((), ()))
NEG = -1000000000.0
A_AFTER = (1, 3, 4, 6, 7, 9, 10, 12, 13, 15, 16, 17, 21, 24, 26)
GQ_AFTER = (17, 21, 23, 25)
GP_AFTER = (21, 23, 25, 27)


def _dot(a, b):
    return jnp.dot(a, b, preferred_element_type=F32)


def _dot_nt(a, b):
    return jax.lax.dot_general(a, b, NT, preferred_element_type=F32)


def _recip(x):
    return pl.reciprocal(x, approx=False, full_range=False)


def _exp_plan():
    item_gate = []
    ng = 0
    for pos in list(range(HB // 2 + 2)) + list(range(20, 28)):
        ng += 6 if pos < HB // 2 else (WOS if pos >= 20 else 0)
        if pos in A_AFTER:
            item_gate.append(ng)
            ng += CH // 64
    while len(item_gate) < NIT:
        item_gate.append(ng)
        ng += CH // 64
    plan = {}
    for k in range(NIT * NPC):
        n = k // NPC
        lo = 0 if n < NCH else item_gate[2 * NCH - 1 - QL] + CH // 64
        g = max(lo, k * ng // (NIT * NPC) - LEAD)
        g = max(lo, min(g, item_gate[n] - 1))
        plan.setdefault(g, []).append(k)
    return plan


def _kernel(x_hbm, wqa_hbm, wka_hbm, wva_hbm, woa_hbm, mem0_hbm, wq_hbm, wk_hbm,
            wv_hbm, wo_hbm, gw_hbm, out_hbm,
            x_v, x0_v, qd_v, wqa_v, woa_v, wkvz_v, gw_v, mem0_v, w_v, wo_v,
            qt_v, ka_v, vt_v, g_v, p0_v, land_v,
            sg0_v, sg1_v, st_v, mx_v, fin_v, ocat_v, o0_v, o7_v, b_v, oa_v,
            sem_x, sem_s, sem_wa, sem_w, sem_wo, sem_out):
    xch = ((0, 2), (2, 6), (6, 8), (8, 12), (12, 16))
    w_hbms = (wq_hbm, wk_hbm, wv_hbm)
    wr = D * HB
    stg_vs = (sg0_v, sg1_v)

    def x_copy(i):
        rs = pl.ds(4 * xch[i][0], 4 * (xch[i][1] - xch[i][0]))
        return pltpu.make_async_copy(x_hbm.at[rs], x_v.at[rs], sem_x.at[i])

    small = [
        pltpu.make_async_copy(wka_hbm, wkvz_v.at[pl.ds(0, DHA)], sem_s.at[0]),
        pltpu.make_async_copy(wva_hbm, wkvz_v.at[pl.ds(DHA, DHA)], sem_s.at[1]),
        pltpu.make_async_copy(gw_hbm, gw_v, sem_s.at[2]),
        pltpu.make_async_copy(mem0_hbm, mem0_v, sem_s.at[3]),
    ]

    def wqa_copy(c):
        cs = pl.ds(c * (D // 2), D // 2)
        return pltpu.make_async_copy(wqa_hbm.at[:, cs], wqa_v.at[:, cs], sem_wa.at[c])

    woa_copy = pltpu.make_async_copy(woa_hbm, woa_v, sem_wa.at[2])

    def w_copy(i, j):
        return pltpu.make_async_copy(
            w_hbms[i].at[pl.ds(j * (wr // 2), wr // 2)],
            land_v.at[pl.ds((2 * i + j) * (wr // 2), wr // 2)], sem_w.at[2 * i + j])

    def w_wait(n):
        dst = land_v.at[pl.ds(pl.multiple_of(n * (wr // 2), wr // 2), wr // 2)]
        pltpu.make_async_copy(dst, dst, sem_w.at[n]).wait()

    def wo_copy(c):
        return pltpu.make_async_copy(wo_hbm.at[:, pl.ds(c * 128, 128)],
                                     land_v.at[pl.ds(c * HB * DHB, HB * DHB)],
                                     sem_wo.at[c])

    x_copy(0).start()
    wqa_copy(0).start()
    for cp in small:
        cp.start()
    wqa_copy(1).start()

    def kvm_rows(kv, hd, r, n):
        return pl.ds(pl.multiple_of(wr + (kv * HB + hd) * (NSEG * M) + r, M), n)

    qscale = (DHA ** -0.5) * math.log2(math.e)

    def xblk(rb):
        return x_v[pl.ds(rb * 4, 4)].reshape(128, D)

    def aproj_kvz(rb):
        kvz = _dot_nt(wkvz_v[...], xblk(rb))
        r0 = pl.multiple_of(rb * 128, 128)
        vt_v[:, pl.ds(r0, 128)] = kvz[DHA:2 * DHA, :].astype(BF16)
        t = jnp.concatenate([kvz, jnp.zeros((48, 128), F32)], axis=0).T
        ka_v[pl.ds(r0, 128), :] = t[:, :DHA].astype(BF16)
        x0 = x_v[pl.ds(rb * 4, 4), 0:M, :].reshape(4 * M, D)
        x0_v[pl.ds(pl.multiple_of(rb * 16, 16), 16), :] = pltpu.bitcast(x0, U32)
        g_v[pl.ds(r0, 128), :] = jnp.broadcast_to(
            jax.nn.sigmoid(t[:, 2 * DHA:2 * DHA + 1]), (128, 128))

    def q_store(rb, b, q):
        qT = q.T.astype(BF16)
        for j in range(4):
            qt_v[rb * 8 + b, :, j * 128:(j + 1) * 128] = qT[j * 32:(j + 1) * 32, :]

    def aproj_q(rb, b, defer=False):
        q = _dot(xblk(rb), wqa_v[:, b * 128:(b + 1) * 128]) * qscale
        if defer:
            qd_v[...] = q
        else:
            q_store(rb, b, q)
        return [q[16 * k:16 * k + 16] for k in range(8)]

    def aproj(rb, extra=None, defer=False):
        aproj_kvz(rb)
        for b in range(8):
            deps = aproj_q(rb, b, defer and b == 7)
            if extra is not None:
                extra(b, deps)

    def relayout(i, g, blk, deps):
        stg = stg_vs[blk]
        base = pl.multiple_of(i * wr + g * 1024 + blk * 512, 512)
        v = pltpu.bitcast(land_v[pl.ds(base, 512), :], U32)
        for k in range(8):
            a = v[32 * k:32 * k + 16]
            b = v[32 * k + 16:32 * k + 32]
            if deps is not None:
                a = jnp.where(deps[k] > jnp.inf, U32(0), a)
            stg[pl.ds(3 * k, 16, stride=25), :] = (a & U32(0xffff)) | (b << 16)
            stg[pl.ds(400 + 3 * k, 16, stride=25), :] = (a >> 16) | (b & U32(0xffff0000))
        r = pl.multiple_of(g * 16 + blk * 8, 8)
        for p in range(16):
            w_v[i, 2 * p, pl.ds(r, 8), :] = stg[pl.ds(25 * p, 8, stride=3), :]
            w_v[i, 2 * p + 1, pl.ds(r, 8), :] = stg[pl.ds(400 + 25 * p, 8, stride=3), :]

    def wo_pack(g):
        v = land_v[pl.ds(pl.multiple_of(g * 1024, 1024), 1024), :]
        wo_v[pl.ds(pl.multiple_of(g * 512, 512), 512), :] = pltpu.bitcast(v, U32)

    def wblk(i, h):
        return pltpu.bitcast(w_v[i, h], BF16)

    x_copy(0).wait()
    wqa_copy(0).wait()
    for i in range(1, len(xch)):
        x_copy(i).start()
    for i in range(2):
        for j in range(2):
            w_copy(i, j).start()
    for rb in range(2):
        for b in range(4):
            aproj_q(rb, b)
    wqa_copy(1).wait()
    for cp in small:
        cp.wait()
    gw = gw_v[...]
    gw_row = jnp.concatenate([gw[r:r + 1, :] for r in range(8)], axis=1)
    wkvz_v[2 * DHA:, :] = jnp.broadcast_to(gw_row, (16, D))
    for rb in range(2):
        aproj_kvz(rb)
    for rb in range(2):
        for b in range(4, 8):
            aproj_q(rb, b, rb == 1 and b == 7)
    x_copy(1).wait()

    def abody0(t, c):
        @pl.when(t == 3)
        def _():
            x_copy(2).wait()
        q_store(t * 2 - 1, 7, qd_v[...])
        aproj(t * 2)
        aproj(t * 2 + 1, defer=True)
        return c
    jax.lax.fori_loop(1, 4, abody0, 0)
    x_copy(3).wait()
    w_copy(0, 0).wait()

    def abody1(t, c):
        @pl.when(t == 2)
        def _():
            x_copy(4).wait()
            w_copy(0, 1).wait()
            w_copy(2, 0).start()
            w_copy(2, 1).start()
        q_store(7 + t * 2, 7, qd_v[...])
        for k in range(2):
            g0 = t * 8 + k * 4
            aproj(8 + t * 2 + k,
                  lambda b, deps, g0=g0: relayout(0, g0 + b // 2, b % 2, deps),
                  defer=k == 1)
        return c
    jax.lax.fori_loop(0, 4, abody1, 0)

    def qk_chunk(u, slot, c, mx, gate=None):
        r0 = c * CH if isinstance(c, int) else pl.multiple_of(c * CH, CH)
        st = _dot(ka_v[pl.ds(r0, CH), :], qt_v[u])
        st_v[slot, pl.ds(r0, CH), :] = st
        cm = jnp.max(st.reshape(CH // 8, 8, 512), axis=0)
        if gate is not None:
            for r in range(0, CH, 64):
                gate(st[r:r + 8, 0:128])
        return cm if mx is None else jnp.maximum(mx, cm)

    for c in range(8):
        wo_copy(c).start()
    woa_copy.start()

    def bulk(i, h):
        x0 = pltpu.bitcast(x0_v[...], BF16)
        y = _dot(x0, wblk(i, h))
        p0_v[i, h] = y.astype(BF16)
        return y

    def bbody0(n, c):
        @pl.when(n % 2 == 0)
        def _():
            w_wait(2 + n // 2)
        y = None
        for hh in range(8):
            h = (n % 4) * 8 + hh
            deps = (None, None) if y is None else [
                [y[b * 256 + k * 32:b * 256 + k * 32 + 16] for k in range(8)]
                for b in range(2)]
            y = bulk(n // 4, h)
            for blk in range(2):
                relayout(n // 4 + 1, h, blk, deps[blk])
        return c
    jax.lax.fori_loop(0, 8, bbody0, 0)
    for c in range(8):
        wo_copy(c).wait()
    mx_v[0] = jnp.full((8, 512), -jnp.inf, F32)

    def bbody1(n, c):
        for hh in range(4):
            bulk(2, n * 4 + hh)
            wo_pack(n * 4 + hh)
            if hh == 1:
                mx_v[0] = qk_chunk(0, 0, n, mx_v[0])
            if hh == 2:
                q_store(S // 128 - 1, 7, qd_v[...])
        return c
    jax.lax.fori_loop(0, 8, bbody1, 0)

    x_v[0, 0:M, :] = mem0_v[...]
    for j in range(2 * HB):
        land_v[wr + j * NSEG * M:wr + j * NSEG * M + 64, :] = jnp.zeros((64, DHB), BF16)

    def pv_exp(slot, r, m8):
        st = st_v[slot, r:r + PR, :].reshape(PR // 8, 8, 512)
        p = jnp.exp2(st - m8[None])
        pk = p.reshape(PR, 512).astype(BF16)
        while p.shape[0] > 1:
            p = p.reshape(p.shape[0] // 2, 2, 8, 512)
            p = p[:, 0] + p[:, 1]
        return p[0], pk

    def colmax(mx):
        return jnp.broadcast_to(jnp.max(mx, axis=0, keepdims=True), (8, 512))

    def a_finish(u, l, acc):
        o = acc * _recip(jnp.sum(l, axis=0, keepdims=True))
        o4 = jnp.concatenate([o[:, j * 128:(j + 1) * 128] for j in range(4)], axis=0)
        qb = u // 8
        b = u % 8
        oa_v[pl.ds(pl.multiple_of(qb * 128, 128), 128),
             pl.ds(pl.multiple_of(b * 128, 128), 128)] = o4.T.astype(BF16)

    mx1 = None
    for c in range(QL - NCH):
        mx1 = qk_chunk(1, 1, c, mx1)
    mx_v[1] = mx1
    fin_v[...] = jnp.ones((40, 512), F32)

    bscale = DHB ** -0.5
    ri = jax.lax.broadcasted_iota(jnp.int32, (SEG, L), 0)
    ci = jax.lax.broadcasted_iota(jnp.int32, (SEG, L), 1)
    mask = (ri < M) | (ci >= SEG) | (ri >= ci)
    gr = jax.lax.broadcasted_iota(jnp.int32, (64, 128), 0)
    gc = jax.lax.broadcasted_iota(jnp.int32, (64, 128), 1)
    gsame = (gr // M) == ((gc % 64) // M)
    gmask = gsame & ((gc < 64) | (gr >= gc - 64))

    def softmax_nonorm(sc):
        p = jnp.exp(sc - jnp.max(sc, axis=1, keepdims=True))
        return p.astype(BF16), _recip(jnp.sum(p, axis=1, keepdims=True))

    def grp_qk(grp, hd):
        rs = pl.ds(pl.multiple_of(grp * 64, 64), 64)
        k = jnp.concatenate([land_v[kvm_rows(0, hd, grp * 64, 64), :],
                             p0_v[1, hd, rs, :]], axis=0)
        sc = _dot_nt(p0_v[0, hd, rs, :], k) * bscale
        sc = jnp.where(gmask, sc, jnp.where(gsame, NEG, -jnp.inf))
        return softmax_nonorm(sc)

    def grp_pv(grp, hd, pr, last=False):
        rs = pl.ds(pl.multiple_of(grp * 64, 64), 64)
        v = jnp.concatenate([land_v[kvm_rows(1, hd, grp * 64, 64), :],
                             p0_v[2, hd, rs, :]], axis=0)
        o = (_dot(pr[0], v) * pr[1]).astype(BF16)
        cs = pl.ds(pl.multiple_of(hd * 128, 128), 128)
        if last:
            o7_v[:, cs] = o
        else:
            o0_v[rs, cs] = o

    plan = _exp_plan()

    def step(s, carry):
        h = x_v[s]
        r0 = pl.multiple_of(s * M, M)
        grp = jnp.maximum(s // 8 - 1, 0)
        gh0 = (s % 8) * 4

        mx = {0: mx_v[0], 1: mx_v[1]}
        m8 = {0: colmax(mx[0])}
        ls = {}
        acc = {}
        pks = {}
        gps = {}
        count = {"gate": 0, "item": 0}

        def gate(dep):
            for k in plan.get(count["gate"], ()):
                n, i = divmod(k, NPC)
                t, c = divmod(n, NCH)
                dep4 = jnp.concatenate([dep] * 4, axis=1)
                m = jnp.where(dep4 > jnp.inf, dep4, m8[t])
                cl, pk = pv_exp(t % 2, c * CH + i * PR, m)
                pks.setdefault(n, []).append(pk)
                ls[t] = cl if t not in ls else ls[t] + cl
            count["gate"] += 1

        def a_item():
            j = count["item"]
            count["item"] += 1
            t, c = divmod(j + QL, NCH)
            u = jnp.minimum(s * 2 + t, NUNIT - 1)
            mx[t] = qk_chunk(u, t % 2, c, mx.get(t), gate)
            if c == NCH - 1:
                m8[t] = colmax(mx[t])
            t, c = divmod(j, NCH)
            o = _dot(vt_v[:, c * CH:(c + 1) * CH], jnp.concatenate(pks.pop(j), axis=0))
            acc[t] = o if t not in acc else acc[t] + o
            if j == NCH - 1:
                a_finish(s * 2, ls[0], acc[0])

        def proj(hd):
            qkv = []
            for i in range(3):
                y = _dot(h, wblk(i, hd))
                gate(y[0:8])
                qkv.append(y.astype(BF16))
            q, k, v = qkv
            land_v[kvm_rows(0, hd, r0, M), :] = k[:M]
            land_v[kvm_rows(1, hd, r0, M), :] = v[:M]
            return q, k, v

        def attn_qk(hd, qkv):
            q, k, v = qkv
            k = jnp.concatenate([k, p0_v[1, hd, pl.ds(r0, M), :]], axis=0)
            v = jnp.concatenate([v, p0_v[2, hd, pl.ds(r0, M), :]], axis=0)
            sc = jnp.where(mask, _dot_nt(q, k) * bscale, NEG)
            return softmax_nonorm(sc) + (v,)

        def attn_pv(hd, prv):
            p, r, v = prv
            o = (_dot(p, v) * r).astype(BF16)
            ocat_v[:, hd * 128:(hd + 1) * 128] = pltpu.bitcast(o, U32)

        def side_work(pos):
            for j in range(4):
                if GP_AFTER[j] == pos:
                    grp_pv(grp, gh0 + j, gps.pop(j))
            for j in range(4):
                if GQ_AFTER[j] == pos:
                    gps[j] = grp_qk(grp, gh0 + j)
            if pos in A_AFTER:
                a_item()

        a_finish(jnp.maximum(s * 2 - 1, 0), fin_v[32:40, :], fin_v[0:32, :])
        projs = {}
        pvs = {}
        for k in range(HB // 2 + 2):
            if k < HB // 2:
                for j in range(2):
                    projs[2 * k + j] = proj(2 * k + j)
            if k >= 2:
                for j in range(2):
                    hd = 2 * (k - 2) + j
                    attn_pv(hd, pvs.pop(hd))
            if 1 <= k <= HB // 2:
                for j in range(2):
                    hd = 2 * (k - 1) + j
                    pvs[hd] = attn_qk(hd, projs.pop(hd))
            side_work(k)
        ys = []
        kw = HB * DHB // WOS
        for c in range(8):
            y = None
            for w in range(WOS):
                oc = pltpu.bitcast(ocat_v[:, w * kw:(w + 1) * kw], BF16)
                wo = pltpu.bitcast(
                    wo_v[c * 2048 + w * kw // 2:c * 2048 + (w + 1) * kw // 2, :], BF16)
                yw = _dot(oc, wo)
                gate(yw[0:8])
                y = yw if y is None else y + yw
            ys.append(y)
            side_work(20 + c)
        y = jnp.concatenate(ys, axis=1)
        b_v[s, M:, :] = y[M:]
        x_v[jnp.minimum(s + 1, NSEG - 1), 0:M, :] = y[:M].astype(BF16)
        while count["item"] < NIT:
            a_item()
        mx_v[0] = mx[2]
        mx_v[1] = mx[3]
        fin_v[0:32, :] = acc[1]
        fin_v[32:40, :] = ls[1]
        return carry

    jax.lax.fori_loop(0, NSEG, step, 0, unroll=2)

    a_finish(NUNIT - 1, fin_v[32:40, :], fin_v[0:32, :])
    woa_copy.wait()
    eb = 256
    neb = S // eb

    def out_copy(i):
        return pltpu.make_async_copy(x_v.at[pl.ds(i * 8, 8)],
                                     out_hbm.at[pl.ds(i * 8, 8)], sem_out.at[i])

    def eblock(i, carry):
        r0 = pl.multiple_of(i * eb, eb)
        s0 = pl.multiple_of(i * 8, 8)
        o0 = o0_v[pl.ds(pl.multiple_of(i * 64, 64), 64), :]
        oa = oa_v[pl.ds(r0, eb), :]
        gps = {}
        hds = [jnp.minimum(i * 5 + j, HB - 1) for j in range(5)]
        for c in range(8):
            cs = slice(c * 128, (c + 1) * 128)
            wo = pltpu.bitcast(wo_v[c * 2048:(c + 1) * 2048, :], BF16)
            b0 = _dot(o0, wo).reshape(8, M, 128)
            b = jnp.concatenate([b0, b_v[pl.ds(s0, 8), M:, cs]], axis=1).reshape(eb, 128)
            if 1 <= c <= 5:
                grp_pv(7, hds[c - 1], gps.pop(c - 1), True)
            a = _dot(oa, woa_v[:, cs])
            g = g_v[pl.ds(r0, eb), :]
            x_v[pl.ds(s0, 8), :, cs] = (
                g * a + (1.0 - g) * b).astype(BF16).reshape(8, SEG, 128)
            if c < 5:
                gps[c] = grp_qk(7, hds[c])
        out_copy(i).start()

        @pl.when(i == neb - 2)
        def _():
            o0_v[pl.ds(7 * 64, 64), :] = o7_v[...]
        return carry

    jax.lax.fori_loop(0, neb, eblock, 0)
    for i in range(neb):
        out_copy(i).wait()


@functools.partial(jax.jit, static_argnames=("B_seg_len",))
def pallas_gated_mix__grouped_kv_mqa__memory_aug_recurrent_mem_tr__prompt_kernel(
    A_x, A_wq, A_wk, A_wv, A_wo, B_x, B_mem0, B_Wq, B_Wk, B_Wv, B_Wo, B_seg_len,
    gate_w,
):
    del B_x
    assert B_seg_len == SEG and A_x.shape == (1, S, D)
    hbm = pl.BlockSpec(memory_space=pl.ANY)
    out = pl.pallas_call(
        _kernel,
        out_shape=jax.ShapeDtypeStruct((NSEG, SEG, D), BF16),
        in_specs=[hbm] * 11,
        out_specs=hbm,
        scratch_shapes=[
            pltpu.VMEM((NSEG, SEG, D), BF16),
            pltpu.VMEM((NSEG * M // 2, D), U32),
            pltpu.VMEM((128, 128), F32),
            pltpu.VMEM((D, D), BF16),
            pltpu.VMEM((D, D), BF16),
            pltpu.VMEM((80, D), BF16),
            pltpu.VMEM((8, 128), BF16),
            pltpu.VMEM((M, D), BF16),
            pltpu.VMEM((3, HB, D // 2, DHB), U32),
            pltpu.VMEM((8 * HB * DHB // 2, 128), U32),
            pltpu.VMEM((NUNIT, DHA, 512), BF16),
            pltpu.VMEM((S, DHA), BF16),
            pltpu.VMEM((DHA, S), BF16),
            pltpu.VMEM((S, 128), F32),
            pltpu.VMEM((3, HB, NSEG * M, DHB), BF16),
            pltpu.VMEM((3 * D * HB, DHB), BF16),
            pltpu.VMEM((832, 128), U32),
            pltpu.VMEM((832, 128), U32),
            pltpu.VMEM((2, S, 512), F32),
            pltpu.VMEM((2, 8, 512), F32),
            pltpu.VMEM((40, 512), F32),
            pltpu.VMEM((SEG // 2, HB * DHB), U32),
            pltpu.VMEM((NSEG * M, HB * DHB), BF16),
            pltpu.VMEM((64, HB * DHB), BF16),
            pltpu.VMEM((NSEG, SEG, D), F32),
            pltpu.VMEM((S, D), BF16),
            pltpu.SemaphoreType.DMA((5,)),
            pltpu.SemaphoreType.DMA((4,)),
            pltpu.SemaphoreType.DMA((3,)),
            pltpu.SemaphoreType.DMA((6,)),
            pltpu.SemaphoreType.DMA((8,)),
            pltpu.SemaphoreType.DMA((8,)),
        ],
        compiler_params=pltpu.CompilerParams(vmem_limit_bytes=127 * 1024 * 1024),
    )(
        A_x.reshape(NSEG, SEG, D), A_wq, A_wk.T, A_wv.T, A_wo, B_mem0.reshape(M, D),
        B_Wq.reshape(D * HB, DHB), B_Wk.reshape(D * HB, DHB),
        B_Wv.reshape(D * HB, DHB), B_Wo.reshape(HB * DHB, D),
        gate_w.reshape(8, 128),
    )
    return out.reshape(1, S, D)
```

```python
import functools
import math

import jax
import jax.numpy as jnp
import jax.experimental.pallas as pl
import jax.experimental.pallas.tpu as pltpu

F32 = jnp.float32
BF16 = jnp.bfloat16
U32 = jnp.uint32

S = 2048
D = 1024
DHA = 32
HB = 32
DHB = 128
M = 8
SEG = 32
NSEG = S // SEG
L = M + SEG
NUNIT = (S // 128) * (D // 128)
CH = 256
NCH = S // CH
NIT = 2 * NCH
NPC = 8
PR = CH // NPC
QL = 10
LEAD = 12
WOS = 4
NT = (((1,), (1,)), ((), ()))
NEG = -1000000000.0
A_AFTER = (1, 3, 4, 6, 7, 9, 10, 12, 13, 15, 16, 17, 21, 24, 26)
GQ_AFTER = (17, 21, 23, 25)
GP_AFTER = (21, 23, 25, 27)


def _dot(a, b):
    return jnp.dot(a, b, preferred_element_type=F32)


def _dot_nt(a, b):
    return jax.lax.dot_general(a, b, NT, preferred_element_type=F32)


def _recip(x):
    return pl.reciprocal(x, approx=False, full_range=False)


def _exp_plan():
    item_gate = []
    ng = 0
    for pos in list(range(HB // 2 + 2)) + list(range(20, 28)):
        ng += 6 if pos < HB // 2 else (WOS if pos >= 20 else 0)
        if pos in A_AFTER:
            item_gate.append(ng)
            ng += CH // 64
    while len(item_gate) < NIT:
        item_gate.append(ng)
        ng += CH // 64
    plan = {}
    for k in range(NIT * NPC):
        n = k // NPC
        lo = 0 if n < NCH else item_gate[2 * NCH - 1 - QL] + CH // 64
        g = max(lo, k * ng // (NIT * NPC) - LEAD)
        g = max(lo, min(g, item_gate[n] - 1))
        plan.setdefault(g, []).append(k)
    return plan


def _kernel(x_hbm, wqa_hbm, wka_hbm, wva_hbm, woa_hbm, mem0_hbm, wq_hbm, wk_hbm,
            wv_hbm, wo_hbm, gw_hbm, out_hbm,
            x_v, x0_v, qd_v, wqa_v, woa_v, wkvz_v, gw_v, mem0_v, w_v, wo_v,
            qt_v, ka_v, vt_v, g_v, p0_v, land_v,
            sg0_v, sg1_v, st_v, mx_v, fin_v, ocat_v, o0_v, o7_v, b_v, oa_v,
            sem_x, sem_s, sem_wa, sem_w, sem_wo, sem_out):
    xch = ((0, 2), (2, 6), (6, 8), (8, 12), (12, 16))
    w_hbms = (wq_hbm, wk_hbm, wv_hbm)
    wr = D * HB
    stg_vs = (sg0_v, sg1_v)

    def x_copy(i):
        rs = pl.ds(4 * xch[i][0], 4 * (xch[i][1] - xch[i][0]))
        return pltpu.make_async_copy(x_hbm.at[rs], x_v.at[rs], sem_x.at[i])

    small = [
        pltpu.make_async_copy(wka_hbm, wkvz_v.at[pl.ds(0, DHA)], sem_s.at[0]),
        pltpu.make_async_copy(wva_hbm, wkvz_v.at[pl.ds(DHA, DHA)], sem_s.at[1]),
        pltpu.make_async_copy(gw_hbm, gw_v, sem_s.at[2]),
        pltpu.make_async_copy(mem0_hbm, mem0_v, sem_s.at[3]),
    ]

    def wqa_copy(c, r):
        cs = pl.ds(c * (D // 2), D // 2)
        rs = pl.ds(r * (D // 4), D // 4)
        return pltpu.make_async_copy(wqa_hbm.at[rs, cs], wqa_v.at[rs, cs],
                                     sem_wa.at[4 * c + r])

    woa_copy = pltpu.make_async_copy(woa_hbm, woa_v, sem_wa.at[8])

    def w_copy(i, j):
        return pltpu.make_async_copy(
            w_hbms[i].at[pl.ds(j * (wr // 2), wr // 2)],
            land_v.at[pl.ds((2 * i + j) * (wr // 2), wr // 2)], sem_w.at[2 * i + j])

    def w_wait(n):
        dst = land_v.at[pl.ds(pl.multiple_of(n * (wr // 2), wr // 2), wr // 2)]
        pltpu.make_async_copy(dst, dst, sem_w.at[n]).wait()

    def wo_copy(c):
        return pltpu.make_async_copy(wo_hbm.at[:, pl.ds(c * 128, 128)],
                                     land_v.at[pl.ds(c * HB * DHB, HB * DHB)],
                                     sem_wo.at[c])

    x_copy(0).start()
    for r in range(4):
        wqa_copy(0, r).start()
    for stg in stg_vs:
        stg[...] = jnp.zeros(stg.shape, U32)

    def kvm_rows(kv, hd, r, n):
        return pl.ds(pl.multiple_of(wr + (kv * HB + hd) * (NSEG * M) + r, M), n)

    qscale = (DHA ** -0.5) * math.log2(math.e)

    def xblk(rb):
        return x_v[pl.ds(rb * 4, 4)].reshape(128, D)

    def aproj_kvz(rb):
        kvz = _dot_nt(wkvz_v[...], xblk(rb))
        r0 = pl.multiple_of(rb * 128, 128)
        vt_v[:, pl.ds(r0, 128)] = kvz[DHA:2 * DHA, :].astype(BF16)
        t = jnp.concatenate([kvz, jnp.zeros((48, 128), F32)], axis=0).T
        ka_v[pl.ds(r0, 128), :] = t[:, :DHA].astype(BF16)
        x0 = x_v[pl.ds(rb * 4, 4), 0:M, :].reshape(4 * M, D)
        x0_v[pl.ds(pl.multiple_of(rb * 16, 16), 16), :] = pltpu.bitcast(x0, U32)
        g_v[pl.ds(r0, 128), :] = jnp.broadcast_to(
            jax.nn.sigmoid(t[:, 2 * DHA:2 * DHA + 1]), (128, 128))

    def q_store(rb, b, q):
        qT = q.T.astype(BF16)
        for j in range(4):
            qt_v[rb * 8 + b, :, j * 128:(j + 1) * 128] = qT[j * 32:(j + 1) * 32, :]

    def aproj_q(rb, b, defer=False):
        q = _dot(xblk(rb), wqa_v[:, b * 128:(b + 1) * 128]) * qscale
        if defer:
            qd_v[...] = q
        else:
            q_store(rb, b, q)
        return [q[16 * k:16 * k + 16] for k in range(8)]

    def aproj(rb, extra=None, defer=False):
        aproj_kvz(rb)
        for b in range(8):
            deps = aproj_q(rb, b, defer and b == 7)
            if extra is not None:
                extra(b, deps)

    def relayout(i, g, blk, deps):
        stg = stg_vs[blk]
        base = pl.multiple_of(i * wr + g * 1024 + blk * 512, 512)
        v = pltpu.bitcast(land_v[pl.ds(base, 512), :], U32)
        for k in range(8):
            a = v[32 * k:32 * k + 16]
            b = v[32 * k + 16:32 * k + 32]
            if deps is not None:
                a = jnp.where(deps[k] > jnp.inf, U32(0), a)
            stg[pl.ds(3 * k, 16, stride=25), :] = (a & U32(0xffff)) | (b << 16)
            stg[pl.ds(400 + 3 * k, 16, stride=25), :] = (a >> 16) | (b & U32(0xffff0000))
        r = pl.multiple_of(g * 16 + blk * 8, 8)
        for p in range(16):
            w_v[i, 2 * p, pl.ds(r, 8), :] = stg[pl.ds(25 * p, 8, stride=3), :]
            w_v[i, 2 * p + 1, pl.ds(r, 8), :] = stg[pl.ds(400 + 25 * p, 8, stride=3), :]

    def wo_pack(g):
        v = land_v[pl.ds(pl.multiple_of(g * 1024, 1024), 1024), :]
        wo_v[pl.ds(pl.multiple_of(g * 512, 512), 512), :] = pltpu.bitcast(v, U32)

    def wblk(i, h):
        return pltpu.bitcast(w_v[i, h], BF16)

    x_copy(0).wait()
    for cp in small:
        cp.start()
    for r in range(4):
        wqa_copy(1, r).start()
    for r in range(4):
        wqa_copy(0, r).wait()
    for i in range(1, len(xch)):
        x_copy(i).start()
    for i in range(2):
        for j in range(2):
            w_copy(i, j).start()
    for rb in range(2):
        for b in range(4):
            aproj_q(rb, b)
    for r in range(4):
        wqa_copy(1, r).wait()
    for cp in small:
        cp.wait()
    gw = gw_v[...]
    gw_row = jnp.concatenate([gw[r:r + 1, :] for r in range(8)], axis=1)
    wkvz_v[2 * DHA:, :] = jnp.broadcast_to(gw_row, (16, D))
    for rb in range(2):
        aproj_kvz(rb)
    for rb in range(2):
        for b in range(4, 8):
            aproj_q(rb, b, rb == 1 and b == 7)
    x_copy(1).wait()

    def abody0(t, c):
        @pl.when(t == 3)
        def _():
            x_copy(2).wait()
        q_store(t * 2 - 1, 7, qd_v[...])
        aproj(t * 2)
        aproj(t * 2 + 1, defer=True)
        return c
    jax.lax.fori_loop(1, 4, abody0, 0)
    x_copy(3).wait()
    w_copy(0, 0).wait()

    def abody1(t, c):
        @pl.when(t == 2)
        def _():
            x_copy(4).wait()
            w_copy(0, 1).wait()
            w_copy(2, 0).start()
            w_copy(2, 1).start()
        q_store(7 + t * 2, 7, qd_v[...])
        for k in range(2):
            g0 = t * 8 + k * 4
            aproj(8 + t * 2 + k,
                  lambda b, deps, g0=g0: relayout(0, g0 + b // 2, b % 2, deps),
                  defer=k == 1)
        return c
    jax.lax.fori_loop(0, 4, abody1, 0)

    def qk_chunk(u, slot, c, mx, gate=None):
        r0 = c * CH if isinstance(c, int) else pl.multiple_of(c * CH, CH)
        st = _dot(ka_v[pl.ds(r0, CH), :], qt_v[u])
        st_v[slot, pl.ds(r0, CH), :] = st
        cm = jnp.max(st.reshape(CH // 8, 8, 512), axis=0)
        if gate is not None:
            for r in range(0, CH, 64):
                gate(st[r:r + 8, 0:128])
        return cm if mx is None else jnp.maximum(mx, cm)

    for c in range(8):
        wo_copy(c).start()
    woa_copy.start()

    def bulk(i, h):
        x0 = pltpu.bitcast(x0_v[...], BF16)
        y = _dot(x0, wblk(i, h))
        p0_v[i, h] = y.astype(BF16)
        return y

    def bbody0(n, c):
        @pl.when(n % 2 == 0)
        def _():
            w_wait(2 + n // 2)
        y = None
        for hh in range(8):
            h = (n % 4) * 8 + hh
            deps = (None, None) if y is None else [
                [y[b * 256 + k * 32:b * 256 + k * 32 + 16] for k in range(8)]
                for b in range(2)]
            y = bulk(n // 4, h)
            for blk in range(2):
                relayout(n // 4 + 1, h, blk, deps[blk])
        return c
    jax.lax.fori_loop(0, 8, bbody0, 0)
    for c in range(8):
        wo_copy(c).wait()
    mx_v[0] = jnp.full((8, 512), -jnp.inf, F32)

    def bbody1(n, c):
        for hh in range(4):
            bulk(2, n * 4 + hh)
            wo_pack(n * 4 + hh)
            if hh == 1:
                mx_v[0] = qk_chunk(0, 0, n, mx_v[0])
            if hh == 2:
                q_store(S // 128 - 1, 7, qd_v[...])
        for j in range(8):
            land_v[kvm_rows(0, n * 8 + j, 0, 64), :] = jnp.zeros((64, DHB), BF16)
        return c
    jax.lax.fori_loop(0, 8, bbody1, 0)

    x_v[0, 0:M, :] = mem0_v[...]

    def pv_exp(slot, r, m8):
        st = st_v[slot, r:r + PR, :].reshape(PR // 8, 8, 512)
        p = jnp.exp2(st - m8[None])
        pk = p.reshape(PR, 512).astype(BF16)
        while p.shape[0] > 1:
            p = p.reshape(p.shape[0] // 2, 2, 8, 512)
            p = p[:, 0] + p[:, 1]
        return p[0], pk

    def colmax(mx):
        return jnp.broadcast_to(jnp.max(mx, axis=0, keepdims=True), (8, 512))

    def a_finish(u, l, acc):
        o = acc * _recip(jnp.sum(l, axis=0, keepdims=True))
        o4 = jnp.concatenate([o[:, j * 128:(j + 1) * 128] for j in range(4)], axis=0)
        qb = u // 8
        b = u % 8
        oa_v[pl.ds(pl.multiple_of(qb * 128, 128), 128),
             pl.ds(pl.multiple_of(b * 128, 128), 128)] = o4.T.astype(BF16)

    mx1 = None
    for c in range(QL - NCH):
        mx1 = qk_chunk(1, 1, c, mx1)
    mx_v[1] = mx1
    fin_v[...] = jnp.ones((40, 512), F32)

    bscale = DHB ** -0.5
    ri = jax.lax.broadcasted_iota(jnp.int32, (SEG, L), 0)
    ci = jax.lax.broadcasted_iota(jnp.int32, (SEG, L), 1)
    mask = (ri < M) | (ci >= SEG) | (ri >= ci)
    gr = jax.lax.broadcasted_iota(jnp.int32, (64, 128), 0)
    gc = jax.lax.broadcasted_iota(jnp.int32, (64, 128), 1)
    gsame = (gr // M) == ((gc % 64) // M)
    gmask = gsame & ((gc < 64) | (gr >= gc - 64))

    def softmax_nonorm(sc):
        p = jnp.exp(sc - jnp.max(sc, axis=1, keepdims=True))
        return p.astype(BF16), _recip(jnp.sum(p, axis=1, keepdims=True))

    def grp_qk(grp, hd):
        rs = pl.ds(pl.multiple_of(grp * 64, 64), 64)
        k = jnp.concatenate([land_v[kvm_rows(0, hd, grp * 64, 64), :],
                             p0_v[1, hd, rs, :]], axis=0)
        sc = _dot_nt(p0_v[0, hd, rs, :], k) * bscale
        sc = jnp.where(gmask, sc, jnp.where(gsame, NEG, -jnp.inf))
        return softmax_nonorm(sc)

    def grp_pv(grp, hd, pr, last=False):
        rs = pl.ds(pl.multiple_of(grp * 64, 64), 64)
        v = jnp.concatenate([land_v[kvm_rows(1, hd, grp * 64, 64), :],
                             p0_v[2, hd, rs, :]], axis=0)
        o = (_dot(pr[0], v) * pr[1]).astype(BF16)
        cs = pl.ds(pl.multiple_of(hd * 128, 128), 128)
        if last:
            o7_v[:, cs] = o
        else:
            o0_v[rs, cs] = o

    plan = _exp_plan()

    def step(s, carry):
        h = x_v[s]
        r0 = pl.multiple_of(s * M, M)
        grp = jnp.maximum(s // 8 - 1, 0)
        gh0 = (s % 8) * 4

        mx = {0: mx_v[0], 1: mx_v[1]}
        m8 = {0: colmax(mx[0])}
        ls = {}
        acc = {}
        pks = {}
        gps = {}
        count = {"gate": 0, "item": 0}

        def gate(dep):
            for k in plan.get(count["gate"], ()):
                n, i = divmod(k, NPC)
                t, c = divmod(n, NCH)
                dep4 = jnp.concatenate([dep] * 4, axis=1)
                m = jnp.where(dep4 > jnp.inf, dep4, m8[t])
                cl, pk = pv_exp(t % 2, c * CH + i * PR, m)
                pks.setdefault(n, []).append(pk)
                ls[t] = cl if t not in ls else ls[t] + cl
            count["gate"] += 1

        def a_item():
            j = count["item"]
            count["item"] += 1
            t, c = divmod(j + QL, NCH)
            u = jnp.minimum(s * 2 + t, NUNIT - 1)
            mx[t] = qk_chunk(u, t % 2, c, mx.get(t), gate)
            if c == NCH - 1:
                m8[t] = colmax(mx[t])
            t, c = divmod(j, NCH)
            o = _dot(vt_v[:, c * CH:(c + 1) * CH], jnp.concatenate(pks.pop(j), axis=0))
            acc[t] = o if t not in acc else acc[t] + o
            if j == NCH - 1:
                a_finish(s * 2, ls[0], acc[0])

        def proj(hd):
            qkv = []
            for i in range(3):
                y = _dot(h, wblk(i, hd))
                gate(y[0:8])
                qkv.append(y.astype(BF16))
            q, k, v = qkv
            land_v[kvm_rows(0, hd, r0, M), :] = k[:M]
            land_v[kvm_rows(1, hd, r0, M), :] = v[:M]
            return q, k, v

        def attn_qk(hd, qkv):
            q, k, v = qkv
            k = jnp.concatenate([k, p0_v[1, hd, pl.ds(r0, M), :]], axis=0)
            v = jnp.concatenate([v, p0_v[2, hd, pl.ds(r0, M), :]], axis=0)
            sc = jnp.where(mask, _dot_nt(q, k) * bscale, NEG)
            return softmax_nonorm(sc) + (v,)

        def attn_pv(hd, prv):
            p, r, v = prv
            o = (_dot(p, v) * r).astype(BF16)
            ocat_v[:, hd * 128:(hd + 1) * 128] = pltpu.bitcast(o, U32)

        def side_work(pos):
            for j in range(4):
                if GP_AFTER[j] == pos:
                    grp_pv(grp, gh0 + j, gps.pop(j))
            for j in range(4):
                if GQ_AFTER[j] == pos:
                    gps[j] = grp_qk(grp, gh0 + j)
            if pos in A_AFTER:
                a_item()

        a_finish(jnp.maximum(s * 2 - 1, 0), fin_v[32:40, :], fin_v[0:32, :])
        projs = {}
        pvs = {}
        for k in range(HB // 2 + 2):
            if k < HB // 2:
                for j in range(2):
                    projs[2 * k + j] = proj(2 * k + j)
            if k >= 2:
                for j in range(2):
                    hd = 2 * (k - 2) + j
                    attn_pv(hd, pvs.pop(hd))
            if 1 <= k <= HB // 2:
                for j in range(2):
                    hd = 2 * (k - 1) + j
                    pvs[hd] = attn_qk(hd, projs.pop(hd))
            side_work(k)
        ys = []
        kw = HB * DHB // WOS
        for c in range(8):
            y = None
            for w in range(WOS):
                oc = pltpu.bitcast(ocat_v[:, w * kw:(w + 1) * kw], BF16)
                wo = pltpu.bitcast(
                    wo_v[c * 2048 + w * kw // 2:c * 2048 + (w + 1) * kw // 2, :], BF16)
                yw = _dot(oc, wo)
                gate(yw[0:8])
                y = yw if y is None else y + yw
            ys.append(y)
            side_work(20 + c)
        y = jnp.concatenate(ys, axis=1)
        b_v[s, M:, :] = y[M:]
        x_v[jnp.minimum(s + 1, NSEG - 1), 0:M, :] = y[:M].astype(BF16)
        while count["item"] < NIT:
            a_item()
        mx_v[0] = mx[2]
        mx_v[1] = mx[3]
        fin_v[0:32, :] = acc[1]
        fin_v[32:40, :] = ls[1]
        return carry

    jax.lax.fori_loop(0, NSEG, step, 0, unroll=2)

    woa_copy.wait()
    eb = 256
    neb = S // eb

    def out_copy(i):
        return pltpu.make_async_copy(x_v.at[pl.ds(i * 8, 8)],
                                     out_hbm.at[pl.ds(i * 8, 8)], sem_out.at[i])

    def eblock(i, carry):
        r0 = pl.multiple_of(i * eb, eb)
        s0 = pl.multiple_of(i * 8, 8)
        o0 = o0_v[pl.ds(pl.multiple_of(i * 64, 64), 64), :]
        oa = oa_v[pl.ds(r0, eb), :]
        gps = {}
        hds = [jnp.minimum(i * 5 + j, HB - 1) for j in range(5)]
        for c in range(8):
            cs = slice(c * 128, (c + 1) * 128)
            wo = pltpu.bitcast(wo_v[c * 2048:(c + 1) * 2048, :], BF16)
            b0 = _dot(o0, wo).reshape(8, M, 128)
            b = jnp.concatenate([b0, b_v[pl.ds(s0, 8), M:, cs]], axis=1).reshape(eb, 128)
            if 1 <= c <= 5:
                grp_pv(7, hds[c - 1], gps.pop(c - 1), True)
            a = _dot(oa, woa_v[:, cs])
            g = g_v[pl.ds(r0, eb), :]
            x_v[pl.ds(s0, 8), :, cs] = (
                g * a + (1.0 - g) * b).astype(BF16).reshape(8, SEG, 128)
            if c < 5:
                gps[c] = grp_qk(7, hds[c])
        out_copy(i).start()

        @pl.when(i == neb - 2)
        def _():
            o0_v[pl.ds(7 * 64, 64), :] = o7_v[...]
            a_finish(NUNIT - 1, fin_v[32:40, :], fin_v[0:32, :])
        return carry

    jax.lax.fori_loop(0, neb, eblock, 0)
    for i in range(neb):
        out_copy(i).wait()


@functools.partial(jax.jit, static_argnames=("B_seg_len",))
def pallas_gated_mix__grouped_kv_mqa__memory_aug_recurrent_mem_tr__prompt_kernel(
    A_x, A_wq, A_wk, A_wv, A_wo, B_x, B_mem0, B_Wq, B_Wk, B_Wv, B_Wo, B_seg_len,
    gate_w,
):
    del B_x
    assert B_seg_len == SEG and A_x.shape == (1, S, D)
    hbm = pl.BlockSpec(memory_space=pl.ANY)
    out = pl.pallas_call(
        _kernel,
        out_shape=jax.ShapeDtypeStruct((NSEG, SEG, D), BF16),
        in_specs=[hbm] * 11,
        out_specs=hbm,
        scratch_shapes=[
            pltpu.VMEM((NSEG, SEG, D), BF16),
            pltpu.VMEM((NSEG * M // 2, D), U32),
            pltpu.VMEM((128, 128), F32),
            pltpu.VMEM((D, D), BF16),
            pltpu.VMEM((D, D), BF16),
            pltpu.VMEM((80, D), BF16),
            pltpu.VMEM((8, 128), BF16),
            pltpu.VMEM((M, D), BF16),
            pltpu.VMEM((3, HB, D // 2, DHB), U32),
            pltpu.VMEM((8 * HB * DHB // 2, 128), U32),
            pltpu.VMEM((NUNIT, DHA, 512), BF16),
            pltpu.VMEM((S, DHA), BF16),
            pltpu.VMEM((DHA, S), BF16),
            pltpu.VMEM((S, 128), F32),
            pltpu.VMEM((3, HB, NSEG * M, DHB), BF16),
            pltpu.VMEM((3 * D * HB, DHB), BF16),
            pltpu.VMEM((832, 128), U32),
            pltpu.VMEM((832, 128), U32),
            pltpu.VMEM((2, S, 512), F32),
            pltpu.VMEM((2, 8, 512), F32),
            pltpu.VMEM((40, 512), F32),
            pltpu.VMEM((SEG // 2, HB * DHB), U32),
            pltpu.VMEM((NSEG * M, HB * DHB), BF16),
            pltpu.VMEM((64, HB * DHB), BF16),
            pltpu.VMEM((NSEG, SEG, D), F32),
            pltpu.VMEM((S, D), BF16),
            pltpu.SemaphoreType.DMA((5,)),
            pltpu.SemaphoreType.DMA((4,)),
            pltpu.SemaphoreType.DMA((9,)),
            pltpu.SemaphoreType.DMA((6,)),
            pltpu.SemaphoreType.DMA((8,)),
            pltpu.SemaphoreType.DMA((8,)),
        ],
        compiler_params=pltpu.CompilerParams(vmem_limit_bytes=127 * 1024 * 1024),
    )(
        A_x.reshape(NSEG, SEG, D), A_wq, A_wk.T, A_wv.T, A_wo, B_mem0.reshape(M, D),
        B_Wq.reshape(D * HB, DHB), B_Wk.reshape(D * HB, DHB),
        B_Wv.reshape(D * HB, DHB), B_Wo.reshape(HB * DHB, D),
        gate_w.reshape(8, 128),
    )
    return out.reshape(1, S, D)
```
